```python
import jax
import jax.numpy as jnp

def _softmax(x, axis=-1):
    return jax.nn.softmax(x, axis=axis)
def _gelu(x):
    return jax.nn.gelu(x, approximate=True)
def _silu(x):
    return jax.nn.silu(x)
def _sigmoid(x):
    return jax.nn.sigmoid(x)
def _layernorm(x, axis=-1, eps=1e-5):
    m = jnp.mean(x, axis=axis, keepdims=True)
    v = jnp.var(x, axis=axis, keepdims=True)
    return (x - m) / jnp.sqrt(v + eps)
def _scatter_add(tgt, idx, src, axis=0):
    return tgt.at[idx].add(src)
def _segment_sum(src, seg, n):
    return jax.ops.segment_sum(src, seg, n)
class _Rng:
    def __init__(self, key):
        self._k = key
    def _next(self):
        self._k, sub = jax.random.split(self._k)
        return sub
    def normal(self, shape):
        return jax.random.normal(self._next(), shape, dtype=jnp.bfloat16)
    def randint(self, lo, hi, shape):
        return jax.random.randint(self._next(), shape, lo, hi, dtype=jnp.int32)
    def uniform(self, shape, lo=0.0, hi=1.0):
        return jax.random.uniform(self._next(), shape, jnp.bfloat16, lo, hi)
    def permutation(self, n):
        return jax.random.permutation(self._next(), n)


kernel_name = 'gated_mix__compressed_kv_cla__gqa_block_cached__decode'

def setup_inputs():
    _rng = _Rng(jax.random.key(int.from_bytes(__import__("os").urandom(4), "little")))
    _w = (lambda a: (lambda t: t.astype(jnp.bfloat16) if jnp.issubdtype(t.dtype, jnp.floating) else t)(jnp.asarray(a)))
    def _A_setup():
        B, H, Sq, Sk, D, M = 1, 32, 1, 4096, 128, 640
        Dc = 4 * D
        return {
            "x": _w((lambda *s: _rng.normal(s) * 0.05)(B, Sq, M)),
            "c_kv": _w((lambda *s: _rng.normal(s) * 0.05)(B, Sk, Dc)),
            "w_q": _w((lambda *s: _rng.normal(s) * 0.05)(M, H, D) * (M ** -0.5)),
            "w_uk": _w((lambda *s: _rng.normal(s) * 0.05)(Dc, H, D) * (Dc ** -0.5)),
            "w_uv": _w((lambda *s: _rng.normal(s) * 0.05)(Dc, H, D) * (Dc ** -0.5)),
            "w_o": _w((lambda *s: _rng.normal(s) * 0.05)(H, D, M) * ((H * D) ** -0.5)),
        }
    _A_in = _A_setup()

    def _B_setup():
        B, Sq, D = 1, 1, 640
        Hq, Hkv, Sk, Dh = 32, 32, 4096, 128
        assert Hq % Hkv == 0, (Hq, Hkv)
        return {
            "x": _w((lambda *s: _rng.normal(s) * 0.05)(B, Sq, D)),
            "k_cache": _w((lambda *s: _rng.normal(s) * 0.05)(B, Hkv, Sk, Dh)),
            "v_cache": _w((lambda *s: _rng.normal(s) * 0.05)(B, Hkv, Sk, Dh)),
            "wq": _w((lambda *s: _rng.normal(s) * 0.05)(D, Hq * Dh) * (D ** -0.5)),
            "wo": _w((lambda *s: _rng.normal(s) * 0.05)(Hq * Dh, D) * ((Hq * Dh) ** -0.5)),
        }
    _B_in = _B_setup()

    return {
        "A_x": _A_in["x"],
        "A_c_kv": _A_in["c_kv"],
        "A_w_q": _A_in["w_q"],
        "A_w_uk": _A_in["w_uk"],
        "A_w_uv": _A_in["w_uv"],
        "A_w_o": _A_in["w_o"],
        "B_x": _B_in["x"],
        "B_k_cache": _B_in["k_cache"],
        "B_v_cache": _B_in["v_cache"],
        "B_wq": _B_in["wq"],
        "B_wo": _B_in["wo"],
        "gate_w": _w((lambda *s: _rng.normal(s) * 0.05)(640)),
    }

def reference(A_x, A_c_kv, A_w_q, A_w_uk, A_w_uv, A_w_o, B_x, B_k_cache, B_v_cache, B_wq, B_wo, gate_w):
    def _A_ref(x, c_kv, w_q, w_uk, w_uv, w_o):
        B, Sq, M = x.shape[0], x.shape[1], x.shape[2]
        Sk = c_kv.shape[1]
        H, D = w_q.shape[1], w_q.shape[2]
        q = jnp.einsum("bqm,mhd->bhqd", x, w_q)
        k = jnp.einsum("bkc,chd->bhkd", c_kv, w_uk)
        v = jnp.einsum("bkc,chd->bhkd", c_kv, w_uv)
        scores = jnp.einsum("bhqd,bhkd->bhqk", q, k) * (D ** -0.5)
        off = Sk - Sq
        qi = jnp.arange(Sq)[:, None]
        kj = jnp.arange(Sk)[None, :]
        cmask = kj <= (qi + off)
        scores = jnp.where(cmask[None, None], scores, -1e9)
        p = _softmax(scores, axis=-1)
        ctx = jnp.einsum("bhqk,bhkd->bhqd", p, v)
        return jnp.einsum("bhqd,hdm->bqm", ctx, w_o)

    def _B_ref(x, k_cache, v_cache, wq, wo):
        B, Sq, D = x.shape
        Hq, Dh = 32, 128
        Hkv = k_cache.shape[1]
        rep = Hq // Hkv
        q = (lambda x, *d: x.transpose(*d))((x @ wq).reshape(B, Sq, Hq, Dh), 0, 2, 1, 3)
        k = jnp.repeat(k_cache, rep, axis=1)
        v = jnp.repeat(v_cache, rep, axis=1)
        scores = jnp.einsum("bhqd,bhkd->bhqk", q, k) * (Dh ** -0.5)
        p = _softmax(scores, axis=-1)
        o = jnp.einsum("bhqk,bhkd->bhqd", p, v)
        return (lambda x, *d: x.transpose(*d))(o, 0, 2, 1, 3).reshape(B, Sq, Hq * Dh) @ wo

    x = A_x
    g = _sigmoid((x * gate_w).sum(-1, keepdims=True))
    a = _A_ref(x, A_c_kv, A_w_q, A_w_uk, A_w_uv, A_w_o)
    b = _B_ref(x, B_k_cache, B_v_cache, B_wq, B_wo)
    return g * a + (1 - g) * b
```

```python
import jax
import jax.numpy as jnp
from jax import lax
import jax.experimental.pallas as pl
import jax.experimental.pallas.tpu as pltpu

F32 = jnp.float32
BF16 = jnp.bfloat16

H = 32
D = 128
S = 4096
M = 640
C = 512
NKV = 4
SCALE = float(D) ** -0.5


def _nt(a, b):
    return lax.dot_general(a, b, (((1,), (1,)), ((), ())), preferred_element_type=F32)


def _nn(a, b):
    return jnp.dot(a, b, preferred_element_type=F32)


def _kernel(xa_hbm, xb_hbm, gw_hbm, ckv_hbm, wqa_hbm, wuk_hbm, wuv_hbm, woa_hbm,
            k_hbm, v_hbm, wqb_hbm, wob_hbm,
            o_ref,
            xa_v, xb_v, gw_v, ckv_v, wqa_v, wuk_v, wuv_v, woa_v, wqb_v, wob_v,
            k_ring, v_ring, q_scr, o_scr, x8_scr,
            sem_w, sem_k, sem_v):
    small = [pltpu.make_async_copy(xa_hbm, xa_v, sem_w.at[0]),
             pltpu.make_async_copy(xb_hbm, xb_v, sem_w.at[1]),
             pltpu.make_async_copy(gw_hbm, gw_v, sem_w.at[2])]
    cp_wqb = pltpu.make_async_copy(wqb_hbm, wqb_v, sem_w.at[3])
    cp_wqa = pltpu.make_async_copy(wqa_hbm, wqa_v, sem_w.at[4])
    cp_wuk = pltpu.make_async_copy(wuk_hbm, wuk_v, sem_w.at[5])
    cp_ckv = pltpu.make_async_copy(ckv_hbm, ckv_v, sem_w.at[6])
    cp_wuv = pltpu.make_async_copy(wuv_hbm, wuv_v, sem_w.at[7])
    cp_woa = pltpu.make_async_copy(woa_hbm, woa_v, sem_w.at[8])
    cp_wob = pltpu.make_async_copy(wob_hbm, wob_v, sem_w.at[9])

    def k_copy(h, slot):
        return pltpu.make_async_copy(k_hbm.at[h], k_ring.at[slot], sem_k.at[slot])

    def v_copy(h, slot):
        return pltpu.make_async_copy(v_hbm.at[h], v_ring.at[slot], sem_v.at[slot])

    cp_wqb.start()
    for c in small:
        c.start()
    cp_wqa.start()
    cp_wuk.start()
    cp_ckv.start()
    cp_wuv.start()
    cp_woa.start()
    for h in range(NKV):
        k_copy(h, h).start()
        v_copy(h, h).start()

    for c in small:
        c.wait()

    xa = xa_v[0].astype(F32)
    xb = xb_v[0]
    gw = gw_v[...].astype(F32).reshape(1, M)
    g = jax.nn.sigmoid(jnp.sum(xa * gw, axis=-1, keepdims=True))

    cp_wqb.wait()
    xb8 = jnp.broadcast_to(xb.astype(F32), (8, M)).astype(BF16)
    qb = _nn(xb8, wqb_v[...])
    for h in range(H):
        q_scr[h] = qb[:, h * D:(h + 1) * D]

    r0 = (lax.broadcasted_iota(jnp.int32, (128, 4096), 1) // H
          == lax.broadcasted_iota(jnp.int32, (128, 4096), 0)).astype(F32).astype(BF16)
    hmask = (lax.broadcasted_iota(jnp.int32, (H, 4096), 1) % H
             == lax.broadcasted_iota(jnp.int32, (H, 4096), 0))

    x8_scr[...] = jnp.zeros((8, 128), F32)
    for j in range(M // 128):
        x8_scr[j:j + 1, :] = xa[:, j * 128:(j + 1) * 128]
    xe = _nn(x8_scr[...].astype(BF16), r0)

    cp_wqa.wait()
    qa = jnp.zeros((H, D), F32)
    for j in range(M // 128):
        xsel = jnp.where(hmask, jnp.broadcast_to(xe[j:j + 1, :], (H, 4096)), 0.0).astype(BF16)
        qa = qa + _nn(xsel, wqa_v[j * 4096:(j + 1) * 4096, :])
    qa = qa.astype(BF16)

    cp_wuk.wait()
    qabs = []
    for j in range(C // 128):
        t = _nt(qa, wuk_v[j * 4096:(j + 1) * 4096, :])
        tm = jnp.where(hmask, t, 0.0).astype(BF16)
        qabs.append(_nt(tm, r0))
    qabs = jnp.concatenate(qabs, axis=1).astype(BF16)

    cp_ckv.wait()
    sa = _nt(qabs, ckv_v[...]) * SCALE
    pa = jnp.exp(sa - jnp.max(sa, axis=-1, keepdims=True))
    la = jnp.sum(pa, axis=-1, keepdims=True)
    cc = (_nn(pa.astype(BF16), ckv_v[...]) / la).astype(BF16)

    cp_wuv.wait()
    ctx = jnp.zeros((H, D), F32)
    for j in range(C // 128):
        ce = _nn(cc[:, j * 128:(j + 1) * 128], r0)
        csel = jnp.where(hmask, ce, 0.0).astype(BF16)
        ctx = ctx + _nn(csel, wuv_v[j * 4096:(j + 1) * 4096, :])

    dmask = (lax.broadcasted_iota(jnp.int32, (H, 4096), 1) // D
             == lax.broadcasted_iota(jnp.int32, (H, 4096), 0))

    def blockdiag(y):
        return jnp.where(dmask, jnp.concatenate([y] * H, axis=1), 0.0).astype(BF16)

    cp_woa.wait()
    out_a = jnp.sum(_nn(blockdiag(ctx), woa_v[...]), axis=0, keepdims=True)

    def body(h, carry):
        slot = h % NKV
        k_copy(h, slot).wait()
        q = q_scr[h].astype(BF16)
        s = _nt(q, k_ring[slot]) * SCALE
        p = jnp.exp(s - jnp.max(s, axis=-1, keepdims=True))
        l = jnp.sum(p, axis=-1, keepdims=True)
        v_copy(h, slot).wait()
        o = _nn(p.astype(BF16), v_ring[slot]) / l
        o_scr[pl.ds(h, 1), :] = o[0:1, :]

        @pl.when(h + NKV < H)
        def _():
            k_copy(h + NKV, slot).start()
            v_copy(h + NKV, slot).start()

        @pl.when(h + NKV == H)
        def _():
            cp_wob.start()
        return carry

    lax.fori_loop(0, H, body, 0)

    cp_wob.wait()
    out_b = jnp.sum(_nn(blockdiag(o_scr[...]), wob_v[...]), axis=0, keepdims=True)
    o_ref[0] = (g * out_a + (1.0 - g) * out_b).astype(o_ref.dtype)


@jax.jit
def pallas_gated_mix__compressed_kv_cla__gqa_block_cached__decode_kernel(
    A_x: jax.Array,
    A_c_kv: jax.Array,
    A_w_q: jax.Array,
    A_w_uk: jax.Array,
    A_w_uv: jax.Array,
    A_w_o: jax.Array,
    B_x: jax.Array,
    B_k_cache: jax.Array,
    B_v_cache: jax.Array,
    B_wq: jax.Array,
    B_wo: jax.Array,
    gate_w: jax.Array,
):
    ckv = A_c_kv.reshape(S, C)
    wqa = A_w_q.reshape(M * H, D)
    wuk = A_w_uk.reshape(C * H, D)
    wuv = A_w_uv.reshape(C * H, D)
    woa = A_w_o.reshape(H * D, M)
    k = B_k_cache.reshape(H, S, D)
    v = B_v_cache.reshape(H, S, D)

    any_spec = pl.BlockSpec(memory_space=pl.ANY)
    return pl.pallas_call(
        _kernel,
        in_specs=[any_spec] * 12,
        out_specs=pl.BlockSpec(memory_space=pltpu.VMEM),
        out_shape=jax.ShapeDtypeStruct((1, 1, M), BF16),
        scratch_shapes=[
            pltpu.VMEM((1, 1, M), BF16),
            pltpu.VMEM((1, 1, M), BF16),
            pltpu.VMEM((M,), BF16),
            pltpu.VMEM((S, C), BF16),
            pltpu.VMEM((M * H, D), BF16),
            pltpu.VMEM((C * H, D), BF16),
            pltpu.VMEM((C * H, D), BF16),
            pltpu.VMEM((H * D, M), BF16),
            pltpu.VMEM((M, H * D), BF16),
            pltpu.VMEM((H * D, M), BF16),
            pltpu.VMEM((NKV, S, D), BF16),
            pltpu.VMEM((NKV, S, D), BF16),
            pltpu.VMEM((H, 8, D), F32),
            pltpu.VMEM((H, D), F32),
            pltpu.VMEM((8, 128), F32),
            pltpu.SemaphoreType.DMA((10,)),
            pltpu.SemaphoreType.DMA((NKV,)),
            pltpu.SemaphoreType.DMA((NKV,)),
        ],
        compiler_params=pltpu.CompilerParams(vmem_limit_bytes=100 * 1024 * 1024),
    )(A_x, B_x, gate_w, ckv, wqa, wuk, wuv, woa, k, v, B_wq, B_wo)
```

```python
import functools
import jax
import jax.numpy as jnp
from jax import lax
import jax.experimental.pallas as pl
import jax.experimental.pallas.tpu as pltpu

F32 = jnp.float32
BF16 = jnp.bfloat16

H = 32
D = 128
S = 4096
M = 640
C = 512
SCALE = float(D) ** -0.5

PCH = [352] * 8 + [320] * 4
POFF = [sum(PCH[:i]) for i in range(len(PCH))]
NP = len(PCH)
NR = 2 * NP
PARTS = [(0, 1408), (1408, 2816), (2816, 4096)]
PART_AFTER = {3: 0, 7: 1, 11: 2}
DEPTH = 24
P0, P1 = 0, 1
NWP = 128
WOA_TAIL = 4
SCOPES = False
H_QA, H_QABS, H_SC, H_CTX = 11, 16, 22, 27


def _nt(a, b):
    return lax.dot_general(a, b, (((1,), (1,)), ((), ())), preferred_element_type=F32)


def _nn(a, b):
    return jnp.dot(a, b, preferred_element_type=F32)


class _NoScope:
    def __enter__(self):
        return self

    def __exit__(self, *a):
        return False


def _scope(name):
    return jax.named_scope(name) if SCOPES else _NoScope()


def shr(k, n):
    return k >> n if isinstance(k, int) else lax.shift_right_logical(k, n)


def par(h):
    return h & 1 if isinstance(h, int) else jnp.bitwise_and(h, 1)


def _kernel(xa_hbm, xb_hbm, gw_hbm, ckv_hbm, wqa_hbm, wuk_hbm, wuv_hbm, woa_hbm,
            k_hbm, v_hbm, wqb_hbm, wob_hbm,
            o_ref,
            xa_v, xb_v, gw_v, ckv_v, wqa_v, wuk_v, wuv_v, woa_v, wqb_v, wob_v,
            k_buf, v_buf, q_scr, s_scr, p_scr, l_scr, o_scr, r0_scr, xe_scr,
            qa_scr, qabs_scr, sa_scr, la_scr, cc_scr, ctx_scr, cf_scr, acca_scr, accb_scr,
            sem_s, sem_k, sem_v, sem_w, sem_wob, sem_woa):
    def k_copy(h, j):
        return pltpu.make_async_copy(k_hbm.at[h, pl.ds(POFF[j], PCH[j])],
                                     k_buf.at[par(h), pl.ds(POFF[j], PCH[j])], sem_k.at[j])

    def v_copy(h, j):
        return pltpu.make_async_copy(v_hbm.at[h, pl.ds(POFF[j], PCH[j])],
                                     v_buf.at[par(h), pl.ds(POFF[j], PCH[j])], sem_v.at[j])

    def row_piece(src, dst, k, rows, sem):
        return pltpu.make_async_copy(src.at[pl.ds(k * rows, rows)], dst.at[pl.ds(k * rows, rows)], sem)

    wtab = [
        (NWP, lambda k: row_piece(wob_hbm, wob_v, k, 32, sem_wob.at[shr(k, 2)])),
        (NWP, lambda k: row_piece(wqa_hbm, wqa_v, k, 160, sem_w.at[0])),
        (NWP, lambda k: row_piece(wuk_hbm, wuk_v, k, 128, sem_w.at[1])),
        (NWP, lambda k: row_piece(ckv_hbm, ckv_v, k, 32, sem_w.at[2])),
        (NWP, lambda k: row_piece(wuv_hbm, wuv_v, k, 128, sem_w.at[3])),
        (NWP - 4 * WOA_TAIL, lambda k: row_piece(woa_hbm, woa_v, k, 32, sem_woa.at[shr(k, 2)])),
    ]

    def w_issue(i):
        arr = shr(i, 7)
        k = jnp.bitwise_and(i, NWP - 1)
        for a, (n, f) in enumerate(wtab):
            cond = (arr == a) if n == NWP else jnp.logical_and(arr == a, k < n)
            @pl.when(cond)
            def _():
                f(k).start(priority=P0)

    def wait_all(buf, sem):
        with _scope("wait_all"):
            pltpu.make_async_copy(buf, buf, sem).wait()

    def wait_head_rows(w_v, sem, k):
        off = k * D if isinstance(k, int) else pl.multiple_of(k * D, D)
        blk = w_v.at[pl.ds(off, D)]
        pltpu.make_async_copy(blk, blk, sem.at[k]).wait()

    def p1_copy(h, r):
        return k_copy(h + 1, r // 2) if r % 2 == 0 else v_copy(h, r // 2)

    small = [pltpu.make_async_copy(xb_hbm, xb_v, sem_s.at[0]),
             pltpu.make_async_copy(xa_hbm, xa_v, sem_s.at[1]),
             pltpu.make_async_copy(gw_hbm, gw_v, sem_s.at[2])]
    cp_wqb = pltpu.make_async_copy(wqb_hbm, wqb_v, sem_s.at[3])
    cp_k0 = pltpu.make_async_copy(k_hbm.at[0], k_buf.at[0], sem_s.at[4])
    for c in small:
        c.start(priority=P0)
    cp_wqb.start(priority=P0)
    cp_k0.start(priority=P1)
    for r in range(DEPTH):
        p1_copy(0, r).start(priority=P1)

    with _scope("r0"):
        r0_scr[...] = (lax.shift_right_logical(lax.broadcasted_iota(jnp.int32, (128, 4096), 1), 5)
                       == lax.broadcasted_iota(jnp.int32, (128, 4096), 0)).astype(F32).astype(BF16)

    def hmask128():
        return (jnp.bitwise_and(lax.broadcasted_iota(jnp.int32, (H, 128), 1), H - 1)
                == lax.broadcasted_iota(jnp.int32, (H, 128), 0))

    def mask_heads(t):
        m = hmask128()
        return jnp.concatenate(
            [jnp.where(m, t[:, b * 128:(b + 1) * 128], 0.0) for b in range(32)], axis=1).astype(BF16)

    acca_scr[...] = jnp.zeros((8, M), F32)
    accb_scr[...] = jnp.zeros((8, M), F32)

    for c in small:
        c.wait()
    xa = xa_v[0].astype(F32)
    gw = gw_v[...].astype(F32).reshape(1, M)
    g = jax.nn.sigmoid(jnp.sum(xa * gw, axis=-1, keepdims=True))
    x8 = jnp.concatenate([xa[:, j * 128:(j + 1) * 128] for j in range(M // 128)]
                         + [jnp.zeros((3, 128), F32)], axis=0)
    xe_scr[...] = _nn(x8.astype(BF16), r0_scr[...])

    with _scope("wait_wqb"):
        cp_wqb.wait()
    with _scope("qb"):
        xb8 = jnp.broadcast_to(xb_v[0].astype(F32), (8, M)).astype(BF16)
        for c4 in range(8):
            qb = _nn(xb8, wqb_v[:, c4 * 512:(c4 + 1) * 512])
            for hh in range(4):
                q_scr[c4 * 4 + hh] = qb[:, hh * D:(hh + 1) * D]

    def qk_part(hn, lo, hi):
        q = q_scr[hn].astype(BF16)
        s_scr[:, lo:hi] = _nt(q, k_buf[par(hn), lo:hi, :])

    def softmax_b():
        s = s_scr[...] * SCALE
        p = jnp.exp(s - jnp.max(s, axis=-1, keepdims=True))
        p_scr[...] = p
        l_scr[...] = jnp.broadcast_to(jnp.sum(p, axis=-1, keepdims=True), (8, D))

    def pv_part(h, part):
        lo, hi = PARTS[part]
        r = _nn(p_scr[:, lo:hi].astype(BF16), v_buf[par(h), lo:hi, :])
        if part == 0:
            o_scr[...] = r
        elif part < len(PARTS) - 1:
            o_scr[...] += r
        else:
            o_scr[...] = (o_scr[...] + r) / l_scr[...]

    def proj_b(h):
        off = h * D if isinstance(h, int) else pl.multiple_of(h * D, D)
        wait_head_rows(wob_v, sem_wob, h)
        accb_scr[...] += _nn(o_scr[...].astype(BF16), wob_v[pl.ds(off, D), :])

    def proj_a(k0, k1):
        def f():
            for k in range(k0, k1):
                wait_head_rows(woa_v, sem_woa, k)
            acca_scr[...] += _nn(cf_scr[:, k0 * D:k1 * D].astype(BF16), woa_v[k0 * D:k1 * D, :])
        return f

    def qa_block(j):
        def f():
            if j == 0:
                wait_all(wqa_v, sem_w.at[0])
            xsel = mask_heads(jnp.broadcast_to(xe_scr[j:j + 1, :], (H, 4096)))
            r = _nn(xsel, wqa_v[j * 4096:(j + 1) * 4096, :])
            if j == 0:
                qa_scr[...] = r
            else:
                qa_scr[...] += r
        return f

    def qabs_block(j):
        def f():
            if j == 0:
                wait_all(wuk_v, sem_w.at[1])
            t = _nt(qa_scr[...].astype(BF16), wuk_v[j * 4096:(j + 1) * 4096, :])
            qabs_scr[:, j * 128:(j + 1) * 128] = _nt(mask_heads(t), r0_scr[...])
        return f

    def sc_block(j):
        def f():
            if j == 0:
                wait_all(ckv_v, sem_w.at[2])
            sa_scr[:, j * 1024:(j + 1) * 1024] = _nt(qabs_scr[...].astype(BF16),
                                                     ckv_v[j * 1024:(j + 1) * 1024, :]) * SCALE
        return f

    def sma_block():
        sa = sa_scr[...]
        pa = jnp.exp(sa - jnp.max(sa, axis=-1, keepdims=True))
        la_scr[...] = jnp.broadcast_to(jnp.sum(pa, axis=-1, keepdims=True), (H, 128))
        sa_scr[...] = pa

    def cc_block(j):
        def f():
            r = _nn(sa_scr[:, j * 1024:(j + 1) * 1024].astype(BF16), ckv_v[j * 1024:(j + 1) * 1024, :])
            if j == 0:
                cc_scr[...] = r
            else:
                cc_scr[...] += r
        return f

    def ctx_block(j):
        def f():
            if j == 0:
                wait_all(wuv_v, sem_w.at[3])
            cc = (cc_scr[:, j * 128:(j + 1) * 128] / la_scr[...]).astype(BF16)
            csel = mask_heads(_nn(cc, r0_scr[...]))
            r = _nn(csel, wuv_v[j * 4096:(j + 1) * 4096, :])
            if j == 0:
                ctx_scr[...] = r
            else:
                ctx_scr[...] += r
        return f

    def flat_block():
        for k in range(H):
            cf_scr[:, k * D:(k + 1) * D] = jnp.broadcast_to(ctx_scr[k:k + 1, :], (8, D))

    sched = {r: [] for r in range(NR)}
    slots = [9, 11, 17, 19, 4]
    for j in range(5):
        sched[slots[j]].append((H_QA + j // 4, qa_block(j)))
    for j in range(4):
        sched[slots[j]].append((H_QABS, qabs_block(j)))
        sched[slots[j]].append((H_SC, sc_block(j)))
        sched[slots[j]].append((H_SC + 1, cc_block(j)))
        sched[slots[j]].append((H_CTX, ctx_block(j)))
    sched[4].append((H_SC + 1, sma_block))
    sched[21].append((H_CTX, flat_block))
    sched[12].append((28, proj_a(0, 6)))
    sched[20].append((28, proj_a(6, 12)))
    sched[20].append((29, proj_a(12, 18)))
    sched[20].append((30, proj_a(18, 24)))

    with _scope("wait_k0"):
        cp_k0.wait()
    qk_part(0, 0, S)

    def body(h, carry):
        for r in range(NR):
            with _scope("wait_p1"):
                p1_copy(h, r).wait()
            with _scope("issue"):
                r2 = r + DEPTH
                if r2 < NR:
                    p1_copy(h, r2).start(priority=P1)
                elif (r2 - NR) % 2 == 1:
                    p1_copy(h + 1, r2 - NR).start(priority=P1)
                else:
                    @pl.when(h + 2 < H)
                    def _():
                        p1_copy(h + 1, r2 - NR).start(priority=P1)
                w_issue(h * NR + r)
            with _scope("compute"):
                if r == 1:
                    softmax_b()
                if r == 3:
                    @pl.when(h > 0)
                    def _():
                        proj_b(h - 1)
                if r % 2 == 0 and r // 2 in PART_AFTER:
                    qk_part(h + 1, *PARTS[PART_AFTER[r // 2]])
                if r % 2 == 1 and r // 2 in PART_AFTER:
                    pv_part(h, PART_AFTER[r // 2])
            with _scope("astage"):
                for hs, f in sched[r]:
                    pl.when(h == hs)(f)
        return carry

    lax.fori_loop(0, H - 1, body, 0)

    h = H - 1
    for j in range(NP):
        with _scope("wait_p1"):
            v_copy(h, j).wait()
        if j + DEPTH // 2 < NP:
            v_copy(h, j + DEPTH // 2).start(priority=P1)
        if j == max(NP - 1 - DEPTH // 2, 0):
            for k in range(H - WOA_TAIL, H):
                row_piece(woa_hbm, woa_v, k, D, sem_woa.at[k]).start(priority=P1)
        w_issue(jnp.int32(h * NR + j))
        if j == 0:
            softmax_b()
        if j == 1:
            proj_b(h - 1)
        if j in PART_AFTER:
            pv_part(h, PART_AFTER[j])
        if j == 10:
            proj_a(24, H - WOA_TAIL)()
    proj_b(h)
    for k in range(H - WOA_TAIL, H):
        with _scope("tail"):
            proj_a(k, k + 1)()

    out = g * acca_scr[0:1, :] + (1.0 - g) * accb_scr[0:1, :]
    o_ref[0] = out.astype(o_ref.dtype)


@jax.jit
def pallas_gated_mix__compressed_kv_cla__gqa_block_cached__decode_kernel(
    A_x, A_c_kv, A_w_q, A_w_uk, A_w_uv, A_w_o, B_x, B_k_cache, B_v_cache, B_wq, B_wo, gate_w,
):
    ckv = A_c_kv.reshape(S, C)
    wqa = A_w_q.reshape(M * H, D)
    wuk = A_w_uk.reshape(C * H, D)
    wuv = A_w_uv.reshape(C * H, D)
    woa = A_w_o.reshape(H * D, M)
    k = B_k_cache.reshape(H, S, D)
    v = B_v_cache.reshape(H, S, D)

    any_spec = pl.BlockSpec(memory_space=pl.ANY)
    return pl.pallas_call(
        _kernel,
        in_specs=[any_spec] * 12,
        out_specs=pl.BlockSpec(memory_space=pltpu.VMEM),
        out_shape=jax.ShapeDtypeStruct((1, 1, M), BF16),
        scratch_shapes=[
            pltpu.VMEM((1, 1, M), BF16),
            pltpu.VMEM((1, 1, M), BF16),
            pltpu.VMEM((M,), BF16),
            pltpu.VMEM((S, C), BF16),
            pltpu.VMEM((M * H, D), BF16),
            pltpu.VMEM((C * H, D), BF16),
            pltpu.VMEM((C * H, D), BF16),
            pltpu.VMEM((H * D, M), BF16),
            pltpu.VMEM((M, H * D), BF16),
            pltpu.VMEM((H * D, M), BF16),
            pltpu.VMEM((2, S, D), BF16),
            pltpu.VMEM((2, S, D), BF16),
            pltpu.VMEM((H, 8, D), F32),
            pltpu.VMEM((8, S), F32),
            pltpu.VMEM((8, S), F32),
            pltpu.VMEM((8, D), F32),
            pltpu.VMEM((8, D), F32),
            pltpu.VMEM((128, 4096), BF16),
            pltpu.VMEM((8, 4096), F32),
            pltpu.VMEM((H, D), F32),
            pltpu.VMEM((H, C), F32),
            pltpu.VMEM((H, S), F32),
            pltpu.VMEM((H, 128), F32),
            pltpu.VMEM((H, C), F32),
            pltpu.VMEM((H, D), F32),
            pltpu.VMEM((8, H * D), F32),
            pltpu.VMEM((8, M), F32),
            pltpu.VMEM((8, M), F32),
            pltpu.SemaphoreType.DMA((5,)),
            pltpu.SemaphoreType.DMA((NP,)),
            pltpu.SemaphoreType.DMA((NP,)),
            pltpu.SemaphoreType.DMA((4,)),
            pltpu.SemaphoreType.DMA((32,)),
            pltpu.SemaphoreType.DMA((32,)),
        ],
        compiler_params=pltpu.CompilerParams(vmem_limit_bytes=100 * 1024 * 1024,
                                             disable_bounds_checks=True,
                                             disable_semaphore_checks=True),
    )(A_x, B_x, gate_w, ckv, wqa, wuk, wuv, woa, k, v, B_wq, B_wo)
```

```python
import functools
import jax
import jax.numpy as jnp
from jax import lax
import jax.experimental.pallas as pl
import jax.experimental.pallas.tpu as pltpu

F32 = jnp.float32
BF16 = jnp.bfloat16

H = 32
D = 128
S = 4096
M = 640
C = 512
SCALE = float(D) ** -0.5


PCH = [320] * 12 + [256]
POFF = [sum(PCH[:i]) for i in range(len(PCH))]
NP = len(PCH)
NR = 2 * NP
PARTS = [(0, 1280), (1280, 2560), (2560, 4096)]
VROT = 0
VSEQ = [(j + VROT) % NP for j in range(NP)]


def _triggers(order):
    trig = {}
    for p, (lo, hi) in enumerate(PARTS):
        need = [j for j in range(NP) if POFF[j] < hi and POFF[j] + PCH[j] > lo]
        trig.setdefault(max(order.index(j) for j in need), []).append(p)
    return trig


K_TRIG = _triggers(list(range(NP)))
V_TRIG = _triggers(VSEQ)
V_ORDER = [p for pos in sorted(V_TRIG) for p in V_TRIG[pos]]
DEPTH = NR
NB = 2
assert DEPTH <= NR * (NB - 1) and DEPTH % 2 == 0
P0, P1 = 0, 1
WOA_TAIL = 4
QROWS = 8
NQP = M // QROWS
PD = 24
NPRO = NQP + NP
W_SKIP = (2, 9, 16, 23)
W_ROUNDS = [r for r in range(NR) if r not in W_SKIP]
NWR = len(W_ROUNDS)
WOP = 32
WQP = 128
WUP = 128
WCP = 32
TAIL_W = 1
SM_ROUND = 1
AG = 2
A_SLOTS = None
MARGIN = 8
PGRP = 3


def _nt(a, b):
    return lax.dot_general(a, b, (((1,), (1,)), ((), ())), preferred_element_type=F32)


def _nn(a, b):
    return jnp.dot(a, b, preferred_element_type=F32)


def shr(k, n):
    return k >> n if isinstance(k, int) else lax.shift_right_logical(k, n)


def band(k, n):
    return k & n if isinstance(k, int) else jnp.bitwise_and(k, n)


def _kernel(xa_hbm, xb_hbm, gw_hbm, ckv_hbm, wqa_hbm, wuk_hbm, wuv_hbm, woa_hbm,
            k_hbm, v_hbm, wqb_hbm, wob_hbm,
            o_ref,
            ckv_v, wqa_v, wuk_v, wuv_v, woa_v, wqb_v, wob_v,
            k_buf, v_buf, q_scr, s_scr, p_scr, l_scr, o_scr, r0_scr, r0t_scr, xe_scr,
            qa_scr, tm_scr, qabs_scr, sa_scr, ma_scr, la_scr, cc_scr, ctx_scr, cf_scr,
            acca_scr, accb_scr, g_scr, xa_v, xb_v, gw_v,
            sem_s, sem_q, sem_k, sem_v, sem_w, sem_wob, sem_woa):
    def k_copy(h, j):
        b = band(h, NB - 1)
        return pltpu.make_async_copy(k_hbm.at[h, pl.ds(POFF[j], PCH[j])],
                                     k_buf.at[b, pl.ds(POFF[j], PCH[j])], sem_k.at[b * NP + j])

    def v_copy(h, j):
        b = band(h, NB - 1)
        return pltpu.make_async_copy(v_hbm.at[h, pl.ds(POFF[j], PCH[j])],
                                     v_buf.at[b, pl.ds(POFF[j], PCH[j])], sem_v.at[b * NP + j])

    def row_piece(src, dst, k, rows, sem):
        return pltpu.make_async_copy(src.at[pl.ds(k * rows, rows)], dst.at[pl.ds(k * rows, rows)], sem)

    def wq_copy(i):
        return row_piece(wqb_hbm, wqb_v, i, QROWS, sem_q.at[i % PD])

    PPH = D // WOP
    SH = PPH.bit_length() - 1
    wtab = [
        (H * PPH, lambda k: row_piece(wob_hbm, wob_v, k, WOP, sem_wob.at[shr(k, SH)])),
        (M * H // WQP, lambda k: row_piece(wqa_hbm, wqa_v, k, WQP, sem_w.at[0])),
        (C * H // WUP, lambda k: row_piece(wuk_hbm, wuk_v, k, WUP, sem_w.at[1])),
        (S // WCP, lambda k: row_piece(ckv_hbm, ckv_v, k, WCP, sem_w.at[2])),
        (C * H // WUP, lambda k: row_piece(wuv_hbm, wuv_v, k, WUP, sem_w.at[3])),
        ((H - WOA_TAIL) * PPH, lambda k: row_piece(woa_hbm, woa_v, k, WOP, sem_woa.at[shr(k, SH)])),
    ]
    wlo = [sum(n for n, _ in wtab[:a]) for a in range(len(wtab) + 1)]
    NW = wlo[-1]
    W_BASE = NPRO
    W_LOOP_END = W_BASE + (H - 1) * NWR
    assert W_LOOP_END + NP * TAIL_W >= NW, (W_LOOP_END + NP * TAIL_W, NW)

    def w_global_round(i):
        k = i - W_BASE
        if k < 0:
            return -1
        return (k // NWR) * NR + W_ROUNDS[k % NWR]

    def w_issue(i):
        if isinstance(i, int):
            for a, (n, f) in enumerate(wtab):
                if wlo[a] <= i < wlo[a + 1]:
                    f(i - wlo[a]).start(priority=P0)
            return
        for a, (n, f) in enumerate(wtab):
            @pl.when(jnp.logical_and(i >= wlo[a], i < wlo[a + 1]))
            def _():
                f(i - wlo[a]).start(priority=P0)

    def wait_all(buf, sem):
        pltpu.make_async_copy(buf, buf, sem).wait()

    def wait_head_rows(w_v, sem, k):
        off = k * D if isinstance(k, int) else pl.multiple_of(k * D, D)
        blk = w_v.at[pl.ds(off, D)]
        pltpu.make_async_copy(blk, blk, sem.at[k]).wait()

    def p1_copy(h, r):
        return k_copy(h + 1, r // 2) if r % 2 == 0 else v_copy(h, VSEQ[r // 2])

    small = [pltpu.make_async_copy(xb_hbm, xb_v, sem_s.at[0]),
             pltpu.make_async_copy(xa_hbm, xa_v, sem_s.at[1]),
             pltpu.make_async_copy(gw_hbm, gw_v, sem_s.at[2])]
    seq = [functools.partial(wq_copy, i) for i in range(NQP)]
    seq += [functools.partial(k_copy, 0, j) for j in range(NP)]
    main = [functools.partial(p1_copy, g // NR, g % NR) for g in range(DEPTH)]
    for i in range(PD):
        seq[i]().start(priority=P1)
    for c in small:
        c.start(priority=P0)

    def hmask128():
        return (jnp.bitwise_and(lax.broadcasted_iota(jnp.int32, (H, 128), 1), H - 1)
                == lax.broadcasted_iota(jnp.int32, (H, 128), 0))

    def mask_heads(t):
        m = hmask128()
        return jnp.concatenate(
            [jnp.where(m, t[:, b * 128:(b + 1) * 128], 0.0) for b in range(t.shape[1] // 128)],
            axis=1).astype(BF16)

    def setup_r0(hf):
        cols = lax.broadcasted_iota(jnp.int32, (128, 2048), 1) + hf * 2048
        r0_scr[:, hf * 2048:(hf + 1) * 2048] = (
            lax.shift_right_logical(cols, 5)
            == lax.broadcasted_iota(jnp.int32, (128, 2048), 0)).astype(F32).astype(BF16)

    def setup_r0t(hf):
        rows = lax.broadcasted_iota(jnp.int32, (2048, 128), 0) + hf * 2048
        r0t_scr[hf * 2048:(hf + 1) * 2048, :] = (
            lax.shift_right_logical(rows, 5)
            == lax.broadcasted_iota(jnp.int32, (2048, 128), 1)).astype(F32).astype(BF16)

    def setup_x():
        acca_scr[...] = jnp.zeros((8, M), F32)
        accb_scr[...] = jnp.zeros((8, M), F32)
        o_scr[...] = jnp.zeros((8, D), F32)
        for c in small:
            c.wait()
        xa = xa_v[0].astype(F32)
        x8 = jnp.concatenate([xa[:, j * 128:(j + 1) * 128] for j in range(M // 128)]
                             + [jnp.zeros((3, 128), F32)], axis=0)
        xe_scr[...] = _nn(x8.astype(BF16), r0_scr[...])
        gw = gw_v[...].astype(F32).reshape(1, M)
        g = jax.nn.sigmoid(jnp.sum(xa * gw, axis=-1, keepdims=True))
        g_scr[...] = jnp.broadcast_to(g, (8, 128))

    def qb_part(blk, half):
        xb8 = jnp.broadcast_to(xb_v[0][:, blk * 128:(blk + 1) * 128].astype(F32), (8, 128)).astype(BF16)
        qb = _nn(xb8, wqb_v[blk * 128:(blk + 1) * 128, half * 2048:(half + 1) * 2048])
        for hh in range(16):
            if blk == 0:
                q_scr[half * 16 + hh] = qb[:, hh * D:(hh + 1) * D]
            else:
                q_scr[half * 16 + hh] += qb[:, hh * D:(hh + 1) * D]

    def qk_part(hn, part):
        lo, hi = PARTS[part]
        q = q_scr[hn].astype(BF16)
        s_scr[:, lo:hi] = _nt(q, k_buf[band(hn, NB - 1), lo:hi, :])

    def softmax_b():
        s = s_scr[...] * SCALE
        p = jnp.exp(s - jnp.max(s, axis=-1, keepdims=True))
        p_scr[...] = p
        l_scr[...] = jnp.broadcast_to(jnp.sum(p, axis=-1, keepdims=True), (8, D))

    def pv_part(h, part):
        lo, hi = PARTS[part]
        r = _nn(p_scr[:, lo:hi].astype(BF16), v_buf[band(h, NB - 1), lo:hi, :])
        if part == V_ORDER[0]:
            o_scr[...] = r
        elif part != V_ORDER[-1]:
            o_scr[...] += r
        else:
            o_scr[...] = (o_scr[...] + r) / l_scr[...]

    def proj_b(h):
        off = h * D if isinstance(h, int) else pl.multiple_of(h * D, D)
        accb_scr[...] += _nn(o_scr[...].astype(BF16), wob_v[pl.ds(off, D), :])

    def proj_a(k0, k1):
        def f():
            for k in range(k0, k1):
                wait_head_rows(woa_v, sem_woa, k)
            acca_scr[...] += _nn(cf_scr[:, k0 * D:k1 * D].astype(BF16), woa_v[k0 * D:k1 * D, :])
        return f

    HB = 2048

    def a_block(wait, fn):
        def f():
            if wait is not None:
                wait_all(*wait)
            fn()
        return f

    def acc(ref, idx, r, first):
        if first:
            ref[idx] = r
        else:
            ref[idx] += r

    def qa_block(j, hf):
        def fn():
            xsel = mask_heads(jnp.broadcast_to(xe_scr[j:j + 1, hf * HB:(hf + 1) * HB], (H, HB)))
            r = _nn(xsel, wqa_v[j * 4096 + hf * HB:j * 4096 + (hf + 1) * HB, :])
            acc(qa_scr, ..., r, j == 0 and hf == 0)
        return a_block((wqa_v, sem_w.at[0]) if j == 0 and hf == 0 else None, fn)

    def qabs_t_block(j, hf):
        def fn():
            t = _nt(qa_scr[...].astype(BF16), wuk_v[j * 4096 + hf * HB:j * 4096 + (hf + 1) * HB, :])
            tm_scr[:, hf * HB:(hf + 1) * HB] = mask_heads(t)
        return a_block((wuk_v, sem_w.at[1]) if j == 0 and hf == 0 else None, fn)

    def qabs_c_block(j, hf):
        def fn():
            r = _nn(tm_scr[:, hf * HB:(hf + 1) * HB], r0t_scr[hf * HB:(hf + 1) * HB, :])
            acc(qabs_scr, (slice(None), slice(j * 128, (j + 1) * 128)), r, hf == 0)
        return a_block(None, fn)

    def sc_block(j):
        def fn():
            sa_scr[:, j * 512:(j + 1) * 512] = _nt(qabs_scr[...].astype(BF16),
                                                   ckv_v[j * 512:(j + 1) * 512, :]) * SCALE
        return a_block((ckv_v, sem_w.at[2]) if j == 0 else None, fn)

    def sma_max():
        ma_scr[...] = jnp.broadcast_to(jnp.max(sa_scr[...], axis=-1, keepdims=True), (H, 128))

    def sma_exp(hf):
        def fn():
            pa = jnp.exp(sa_scr[:, hf * HB:(hf + 1) * HB] - ma_scr[:, 0:1])
            sa_scr[:, hf * HB:(hf + 1) * HB] = pa
            acc(la_scr, ..., jnp.broadcast_to(jnp.sum(pa, axis=-1, keepdims=True), (H, 128)), hf == 0)
        return a_block(None, fn)

    def cc_block(j):
        def fn():
            r = _nn(sa_scr[:, j * 512:(j + 1) * 512].astype(BF16), ckv_v[j * 512:(j + 1) * 512, :])
            acc(cc_scr, ..., r, j == 0)
        return a_block(None, fn)

    def ctx_e_block(j, hf):
        def fn():
            cc = (cc_scr[:, j * 128:(j + 1) * 128] / la_scr[...]).astype(BF16)
            tm_scr[:, hf * HB:(hf + 1) * HB] = mask_heads(_nn(cc, r0_scr[:, hf * HB:(hf + 1) * HB]))
        return a_block((wuv_v, sem_w.at[3]) if j == 0 and hf == 0 else None, fn)

    def ctx_m_block(j, hf):
        def fn():
            r = _nn(tm_scr[:, hf * HB:(hf + 1) * HB],
                    wuv_v[j * 4096 + hf * HB:j * 4096 + (hf + 1) * HB, :])
            acc(ctx_scr, ..., r, j == 0 and hf == 0)
        return a_block(None, fn)

    def flat_block():
        for k in range(H):
            cf_scr[:, k * D:(k + 1) * D] = jnp.broadcast_to(ctx_scr[k:k + 1, :], (8, D))

    b_rounds = {SM_ROUND} | {2 * pos + 1 for pos in V_TRIG} | {2 * pos + 1 for pos in K_TRIG}
    free = [r for r in range(NR) if r not in b_rounds and r - 1 not in b_rounds]
    slots = A_SLOTS if A_SLOTS is not None else free[1::2]
    sched = {r: [] for r in range(NR)}

    def grp(fs):
        def f():
            for x in fs:
                x()
        return f

    def place(blocks, after_piece, start, allowed, group=AG):
        g = max(w_global_round(after_piece) + MARGIN, start)
        blocks = [grp(blocks[i:i + group]) for i in range(0, len(blocks), group)]
        for b in blocks:
            while g % NR not in allowed:
                g += 1
            assert g // NR < H - 1
            sched[g % NR].append((g // NR, b))
            g += 1
        return g

    g = place([qa_block(j, hf) for j in range(5) for hf in range(2)], wlo[2] - 1, 0, slots)
    g = place([blk for j in range(4) for blk in (qabs_t_block(j, 0), qabs_t_block(j, 1),
                                                 qabs_c_block(j, 0), qabs_c_block(j, 1))],
              wlo[3] - 1, g, slots)
    g = place([sc_block(j) for j in range(8)]
              + [a_block(None, sma_max), sma_exp(0), sma_exp(1)]
              + [cc_block(j) for j in range(8)], wlo[4] - 1, g, slots)
    g = place([blk for j in range(4) for blk in (ctx_e_block(j, 0), ctx_e_block(j, 1),
                                                 ctx_m_block(j, 0), ctx_m_block(j, 1))]
              + [a_block(None, flat_block)], wlo[5] - 1, g, slots)
    k_rest = 0
    while k_rest < H - WOA_TAIL:
        k1 = min(k_rest + PGRP, H - WOA_TAIL)
        last = wlo[5] + PPH * k1 - 1
        if last >= W_LOOP_END:
            break
        g2 = max(g, w_global_round(last) + MARGIN)
        while g2 % NR not in free:
            g2 += 1
        if g2 // NR >= H - 1:
            break
        sched[g2 % NR].append((g2 // NR, proj_a(k_rest, k1)))
        g = g2 + 1
        k_rest = k1

    PB = 128 // QROWS
    allseq = seq + main
    for i in range(NPRO):
        seq[i]().wait()
        if i + PD < len(allseq):
            allseq[i + PD]().start(priority=P1)
        if i >= NPRO - (DEPTH - PD) and DEPTH > PD:
            allseq[NPRO + PD + (i - (NPRO - (DEPTH - PD)))]().start(priority=P1)
        w_issue(i)
        if i in (0, 1):
            setup_r0(i)
        if i in (2, 3):
            setup_r0t(i - 2)
        if i == 4:
            setup_x()
        if PB - 1 <= i <= NQP and i % PB in (PB - 1, 0):
            qb_part((i - PB + 1) // PB, 0 if i % PB == PB - 1 else 1)
        for p in K_TRIG.get(i - NQP, []):
            qk_part(0, p)

    def body(h, carry):
        for r in range(NR):
            p1_copy(h, r).wait()
            dh, r2 = divmod(r + DEPTH, NR)
            lim = H - 1 - dh if r2 % 2 == 0 else H - dh
            if lim >= H - 1:
                p1_copy(h + dh, r2).start(priority=P1)
            else:
                @pl.when(h < lim)
                def _():
                    p1_copy(h + dh, r2).start(priority=P1)
            if r in W_ROUNDS:
                w_issue(W_BASE + h * NWR + W_ROUNDS.index(r))
            if r == 0:
                wait_head_rows(wob_v, sem_wob, h)
            if r == SM_ROUND:
                softmax_b()
                proj_b(jnp.maximum(h - 1, 0))
            if r % 2 == 1:
                for p in K_TRIG.get(r // 2, []):
                    qk_part(h + 1, p)
                for p in V_TRIG.get(r // 2, []):
                    pv_part(h, p)
            if sched[r]:
                mask = sum(1 << hs for hs in {hs for hs, _ in sched[r]})

                @pl.when(jnp.bitwise_and(lax.shift_right_logical(jnp.int32(mask), h), 1) == 1)
                def _():
                    for hs, f in sched[r]:
                        pl.when(h == hs)(f)
        return carry

    lax.fori_loop(0, H - 1, body, 0)

    h = H - 1
    issued = set()
    for gidx in range(DEPTH, (H - 1) * NR + DEPTH):
        if gidx // NR == h and gidx % 2 == 1:
            issued.add((gidx % NR) // 2)
    for gidx in range(DEPTH):
        if gidx // NR == h and gidx % 2 == 1:
            issued.add((gidx % NR) // 2)
    pending = [j for j in range(NP) if j not in issued]

    def start_tail():
        for k in range(H - WOA_TAIL, H):
            row_piece(woa_hbm, woa_v, k, D, sem_woa.at[k]).start(priority=P1)

    if not pending:
        start_tail()
    wi = W_LOOP_END
    k_next = k_rest
    w_round = {}
    for j in range(NP):
        v_copy(h, VSEQ[j]).wait()
        if pending:
            v_copy(h, VSEQ[pending.pop(0)]).start(priority=P1)
            if not pending:
                start_tail()
        for _ in range(TAIL_W):
            if wi < NW:
                w_issue(wi)
                w_round[wi] = j
                wi += 1
        if j == 0:
            wait_head_rows(wob_v, sem_wob, h)
            softmax_b()
            proj_b(h - 1)
        if j in V_TRIG:
            for p in V_TRIG[j]:
                pv_part(h, p)
        elif j >= 1:
            k1 = k_next
            while (k1 < H - WOA_TAIL and k1 < k_next + PGRP and wlo[5] + PPH * (k1 + 1) - 1 < wi
                   and w_round.get(wlo[5] + PPH * (k1 + 1) - 1, -100) <= j - 4):
                k1 += 1
            if k1 > k_next:
                proj_a(k_next, k1)()
                k_next = k1
    assert wi >= NW
    proj_b(h)
    if k_next < H - WOA_TAIL:
        proj_a(k_next, H - WOA_TAIL)()
    for k in range(H - WOA_TAIL, H):
        proj_a(k, k + 1)()

    g = g_scr[0:1, 0:1]
    out = g * acca_scr[0:1, :] + (1.0 - g) * accb_scr[0:1, :]
    o_ref[0] = out.astype(o_ref.dtype)


@jax.jit
def pallas_gated_mix__compressed_kv_cla__gqa_block_cached__decode_kernel(
    A_x, A_c_kv, A_w_q, A_w_uk, A_w_uv, A_w_o, B_x, B_k_cache, B_v_cache, B_wq, B_wo, gate_w,
):
    ckv = A_c_kv.reshape(S, C)
    wqa = A_w_q.reshape(M * H, D)
    wuk = A_w_uk.reshape(C * H, D)
    wuv = A_w_uv.reshape(C * H, D)
    woa = A_w_o.reshape(H * D, M)
    k = B_k_cache.reshape(H, S, D)
    v = B_v_cache.reshape(H, S, D)

    any_spec = pl.BlockSpec(memory_space=pl.ANY)
    return pl.pallas_call(
        _kernel,
        in_specs=[any_spec] * 12,
        out_specs=pl.BlockSpec(memory_space=pltpu.VMEM),
        out_shape=jax.ShapeDtypeStruct((1, 1, M), BF16),
        scratch_shapes=[
            pltpu.VMEM((S, C), BF16),
            pltpu.VMEM((M * H, D), BF16),
            pltpu.VMEM((C * H, D), BF16),
            pltpu.VMEM((C * H, D), BF16),
            pltpu.VMEM((H * D, M), BF16),
            pltpu.VMEM((M, H * D), BF16),
            pltpu.VMEM((H * D, M), BF16),
            pltpu.VMEM((NB, S, D), BF16),
            pltpu.VMEM((NB, S, D), BF16),
            pltpu.VMEM((H, 8, D), F32),
            pltpu.VMEM((8, S), F32),
            pltpu.VMEM((8, S), F32),
            pltpu.VMEM((8, D), F32),
            pltpu.VMEM((8, D), F32),
            pltpu.VMEM((128, 4096), BF16),
            pltpu.VMEM((4096, 128), BF16),
            pltpu.VMEM((8, 4096), F32),
            pltpu.VMEM((H, D), F32),
            pltpu.VMEM((H, 4096), BF16),
            pltpu.VMEM((H, C), F32),
            pltpu.VMEM((H, S), F32),
            pltpu.VMEM((H, 128), F32),
            pltpu.VMEM((H, 128), F32),
            pltpu.VMEM((H, C), F32),
            pltpu.VMEM((H, D), F32),
            pltpu.VMEM((8, H * D), F32),
            pltpu.VMEM((8, M), F32),
            pltpu.VMEM((8, M), F32),
            pltpu.VMEM((8, 128), F32),
            pltpu.VMEM((1, 1, M), BF16),
            pltpu.VMEM((1, 1, M), BF16),
            pltpu.VMEM((M,), BF16),
            pltpu.SemaphoreType.DMA((3,)),
            pltpu.SemaphoreType.DMA((PD,)),
            pltpu.SemaphoreType.DMA((NB * NP,)),
            pltpu.SemaphoreType.DMA((NB * NP,)),
            pltpu.SemaphoreType.DMA((4,)),
            pltpu.SemaphoreType.DMA((32,)),
            pltpu.SemaphoreType.DMA((32,)),
        ],
        compiler_params=pltpu.CompilerParams(vmem_limit_bytes=100 * 1024 * 1024,
                                             disable_bounds_checks=True,
                                             disable_semaphore_checks=True),
    )(A_x, B_x, gate_w, ckv, wqa, wuk, wuv, woa, k, v, B_wq, B_wo)
```

```python
import functools
import jax
import jax.numpy as jnp
from jax import lax
import jax.experimental.pallas as pl
import jax.experimental.pallas.tpu as pltpu

F32 = jnp.float32
BF16 = jnp.bfloat16

H = 32
D = 128
S = 4096
M = 640
C = 512
SCALE = float(D) ** -0.5


PCH = [320] * 10 + [256] + [320] * 2
POFF = [sum(PCH[:i]) for i in range(len(PCH))]
NP = len(PCH)
NR = 2 * NP
PARTS = [(0, 1280), (1280, 2560), (2560, 4096)]
VROT = 4
VSEQ = [(j + VROT) % NP for j in range(NP)]


def _triggers(order):
    trig = {}
    for p, (lo, hi) in enumerate(PARTS):
        need = [j for j in range(NP) if POFF[j] < hi and POFF[j] + PCH[j] > lo]
        trig.setdefault(max(order.index(j) for j in need), []).append(p)
    return trig


K_TRIG = _triggers(list(range(NP)))
V_TRIG = _triggers(VSEQ)
V_ORDER = [p for pos in sorted(V_TRIG) for p in V_TRIG[pos]]
DEPTH = NR
NB = 2
assert DEPTH <= NR * (NB - 1) and DEPTH % 2 == 0
P0, P1 = 0, 1
WOA_TAIL = 4
QROWS = 8
NQP = M // QROWS
PD = 32
NPRO = NQP + NP
W_SKIP = (2, 9, 16, 23)
W_ROUNDS = [r for r in range(NR) if r not in W_SKIP]
NWR = len(W_ROUNDS)
WOP = 32
WQP = 128
WUP = 128
WCP = 32
TAIL_W = 1
SM_ROUND = 1
AG = 2
A_SLOTS = None
MARGIN = 8
PGRP = 3
W_FIRST = 0
LASTR = 0
LAST_VPU = 0


def _nt(a, b):
    return lax.dot_general(a, b, (((1,), (1,)), ((), ())), preferred_element_type=F32)


def _nn(a, b):
    return jnp.dot(a, b, preferred_element_type=F32)


def shr(k, n):
    return k >> n if isinstance(k, int) else lax.shift_right_logical(k, n)


def band(k, n):
    return k & n if isinstance(k, int) else jnp.bitwise_and(k, n)


def _kernel(xa_hbm, xb_hbm, gw_hbm, ckv_hbm, wqa_hbm, wuk_hbm, wuv_hbm, woa_hbm,
            k_hbm, v_hbm, wqb_hbm, wob_hbm,
            o_ref,
            ckv_v, wqa_v, wuk_v, wuv_v, woa_v, wqb_v, wob_v,
            k_buf, v_buf, q_scr, s_scr, p_scr, l_scr, o_scr, r0_scr, r0t_scr, xe_scr,
            qa_scr, tm_scr, qabs_scr, sa_scr, ma_scr, la_scr, cc_scr, ctx_scr, cf_scr,
            acca_scr, accb_scr, g_scr, xa_v, xb_v, gw_v,
            sem_s, sem_q, sem_k, sem_v, sem_w, sem_wob, sem_woa):
    def k_copy(h, j):
        b = band(h, NB - 1)
        return pltpu.make_async_copy(k_hbm.at[h, pl.ds(POFF[j], PCH[j])],
                                     k_buf.at[b, pl.ds(POFF[j], PCH[j])], sem_k.at[b * NP + j])

    def v_copy(h, j):
        b = band(h, NB - 1)
        return pltpu.make_async_copy(v_hbm.at[h, pl.ds(POFF[j], PCH[j])],
                                     v_buf.at[b, pl.ds(POFF[j], PCH[j])], sem_v.at[b * NP + j])

    def row_piece(src, dst, k, rows, sem):
        return pltpu.make_async_copy(src.at[pl.ds(k * rows, rows)], dst.at[pl.ds(k * rows, rows)], sem)

    def wq_copy(i):
        return row_piece(wqb_hbm, wqb_v, i, QROWS, sem_q.at[i % PD])

    PPH = D // WOP
    SH = PPH.bit_length() - 1
    wtab = [
        (H * PPH, lambda k: row_piece(wob_hbm, wob_v, k, WOP, sem_wob.at[shr(k, SH)])),
        (M * H // WQP, lambda k: row_piece(wqa_hbm, wqa_v, k, WQP, sem_w.at[0])),
        (C * H // WUP, lambda k: row_piece(wuk_hbm, wuk_v, k, WUP, sem_w.at[1])),
        (S // WCP, lambda k: row_piece(ckv_hbm, ckv_v, k, WCP, sem_w.at[2])),
        (C * H // WUP, lambda k: row_piece(wuv_hbm, wuv_v, k, WUP, sem_w.at[3])),
        ((H - WOA_TAIL) * PPH, lambda k: row_piece(woa_hbm, woa_v, k, WOP, sem_woa.at[shr(k, SH)])),
    ]
    wlo = [sum(n for n, _ in wtab[:a]) for a in range(len(wtab) + 1)]
    NW = wlo[-1]
    W_BASE = NPRO
    W_LOOP_END = W_BASE + (H - 1) * NWR
    assert W_LOOP_END + NP * TAIL_W >= NW, (W_LOOP_END + NP * TAIL_W, NW)

    def w_global_round(i):
        k = i - W_BASE
        if k < 0:
            return -1
        return (k // NWR) * NR + W_ROUNDS[k % NWR]

    def w_issue(i):
        if isinstance(i, int):
            for a, (n, f) in enumerate(wtab):
                if wlo[a] <= i < wlo[a + 1]:
                    f(i - wlo[a]).start(priority=P0)
            return
        for a, (n, f) in enumerate(wtab):
            @pl.when(jnp.logical_and(i >= wlo[a], i < wlo[a + 1]))
            def _():
                f(i - wlo[a]).start(priority=P0)

    def wait_all(buf, sem):
        pltpu.make_async_copy(buf, buf, sem).wait()

    def wait_head_rows(w_v, sem, k):
        off = k * D if isinstance(k, int) else pl.multiple_of(k * D, D)
        blk = w_v.at[pl.ds(off, D)]
        pltpu.make_async_copy(blk, blk, sem.at[k]).wait()

    def p1_copy(h, r):
        return k_copy(h + 1, r // 2) if r % 2 == 0 else v_copy(h, VSEQ[r // 2])

    small = [pltpu.make_async_copy(xb_hbm, xb_v, sem_s.at[0]),
             pltpu.make_async_copy(xa_hbm, xa_v, sem_s.at[1]),
             pltpu.make_async_copy(gw_hbm, gw_v, sem_s.at[2])]
    seq = [functools.partial(wq_copy, i) for i in range(NQP)]
    seq += [functools.partial(k_copy, 0, j) for j in range(NP)]
    main = [functools.partial(p1_copy, g // NR, g % NR) for g in range(DEPTH)]
    for i in range(PD):
        seq[i]().start(priority=P1)
    for c in small:
        c.start(priority=P0)

    def hmask128():
        return (jnp.bitwise_and(lax.broadcasted_iota(jnp.int32, (H, 128), 1), H - 1)
                == lax.broadcasted_iota(jnp.int32, (H, 128), 0))

    def mask_heads(t):
        m = hmask128()
        return jnp.concatenate(
            [jnp.where(m, t[:, b * 128:(b + 1) * 128], 0.0) for b in range(t.shape[1] // 128)],
            axis=1).astype(BF16)

    def setup_r0(hf):
        cols = lax.broadcasted_iota(jnp.int32, (128, 2048), 1) + hf * 2048
        r0_scr[:, hf * 2048:(hf + 1) * 2048] = (
            lax.shift_right_logical(cols, 5)
            == lax.broadcasted_iota(jnp.int32, (128, 2048), 0)).astype(F32).astype(BF16)

    def setup_r0t(hf):
        rows = lax.broadcasted_iota(jnp.int32, (2048, 128), 0) + hf * 2048
        r0t_scr[hf * 2048:(hf + 1) * 2048, :] = (
            lax.shift_right_logical(rows, 5)
            == lax.broadcasted_iota(jnp.int32, (2048, 128), 1)).astype(F32).astype(BF16)

    def setup_x():
        acca_scr[...] = jnp.zeros((8, M), F32)
        accb_scr[...] = jnp.zeros((8, M), F32)
        o_scr[...] = jnp.zeros((8, D), F32)
        for c in small:
            c.wait()
        xa = xa_v[0].astype(F32)
        x8 = jnp.concatenate([xa[:, j * 128:(j + 1) * 128] for j in range(M // 128)]
                             + [jnp.zeros((3, 128), F32)], axis=0)
        xe_scr[...] = _nn(x8.astype(BF16), r0_scr[...])
        gw = gw_v[...].astype(F32).reshape(1, M)
        g = jax.nn.sigmoid(jnp.sum(xa * gw, axis=-1, keepdims=True))
        g_scr[...] = jnp.broadcast_to(g, (8, 128))

    def qb_part(blk, half):
        xb8 = jnp.broadcast_to(xb_v[0][:, blk * 128:(blk + 1) * 128].astype(F32), (8, 128)).astype(BF16)
        qb = _nn(xb8, wqb_v[blk * 128:(blk + 1) * 128, half * 2048:(half + 1) * 2048])
        for hh in range(16):
            if blk == 0:
                q_scr[half * 16 + hh] = qb[:, hh * D:(hh + 1) * D]
            else:
                q_scr[half * 16 + hh] += qb[:, hh * D:(hh + 1) * D]

    def qk_part(hn, part):
        lo, hi = PARTS[part]
        q = q_scr[hn].astype(BF16)
        s_scr[:, lo:hi] = _nt(q, k_buf[band(hn, NB - 1), lo:hi, :])

    def softmax_b():
        s = s_scr[...] * SCALE
        p = jnp.exp(s - jnp.max(s, axis=-1, keepdims=True))
        p_scr[...] = p
        l_scr[...] = jnp.broadcast_to(jnp.sum(p, axis=-1, keepdims=True), (8, D))

    def pv_part(h, part):
        lo, hi = PARTS[part]
        r = _nn(p_scr[:, lo:hi].astype(BF16), v_buf[band(h, NB - 1), lo:hi, :])
        if part == V_ORDER[0]:
            o_scr[...] = r
        elif part != V_ORDER[-1]:
            o_scr[...] += r
        else:
            o_scr[...] = (o_scr[...] + r) / l_scr[...]

    def proj_b(h):
        off = h * D if isinstance(h, int) else pl.multiple_of(h * D, D)
        accb_scr[...] += _nn(o_scr[...].astype(BF16), wob_v[pl.ds(off, D), :])

    def proj_a(k0, k1):
        def f():
            for k in range(k0, k1):
                wait_head_rows(woa_v, sem_woa, k)
            acca_scr[...] += _nn(cf_scr[:, k0 * D:k1 * D].astype(BF16), woa_v[k0 * D:k1 * D, :])
        return f

    HB = 2048

    def a_block(wait, fn):
        def f():
            if wait is not None:
                wait_all(*wait)
            fn()
        return f

    def acc(ref, idx, r, first):
        if first:
            ref[idx] = r
        else:
            ref[idx] += r

    def qa_block(j, hf):
        def fn():
            xsel = mask_heads(jnp.broadcast_to(xe_scr[j:j + 1, hf * HB:(hf + 1) * HB], (H, HB)))
            r = _nn(xsel, wqa_v[j * 4096 + hf * HB:j * 4096 + (hf + 1) * HB, :])
            acc(qa_scr, ..., r, j == 0 and hf == 0)
        return a_block((wqa_v, sem_w.at[0]) if j == 0 and hf == 0 else None, fn)

    def qabs_t_block(j, hf):
        def fn():
            t = _nt(qa_scr[...].astype(BF16), wuk_v[j * 4096 + hf * HB:j * 4096 + (hf + 1) * HB, :])
            tm_scr[:, hf * HB:(hf + 1) * HB] = mask_heads(t)
        return a_block((wuk_v, sem_w.at[1]) if j == 0 and hf == 0 else None, fn)

    def qabs_c_block(j, hf):
        def fn():
            r = _nn(tm_scr[:, hf * HB:(hf + 1) * HB], r0t_scr[hf * HB:(hf + 1) * HB, :])
            acc(qabs_scr, (slice(None), slice(j * 128, (j + 1) * 128)), r, hf == 0)
        return a_block(None, fn)

    def sc_block(j):
        def fn():
            sa_scr[:, j * 512:(j + 1) * 512] = _nt(qabs_scr[...].astype(BF16),
                                                   ckv_v[j * 512:(j + 1) * 512, :]) * SCALE
        return a_block((ckv_v, sem_w.at[2]) if j == 0 else None, fn)

    def sma_max():
        ma_scr[...] = jnp.broadcast_to(jnp.max(sa_scr[...], axis=-1, keepdims=True), (H, 128))

    def sma_exp(hf):
        def fn():
            pa = jnp.exp(sa_scr[:, hf * HB:(hf + 1) * HB] - ma_scr[:, 0:1])
            sa_scr[:, hf * HB:(hf + 1) * HB] = pa
            acc(la_scr, ..., jnp.broadcast_to(jnp.sum(pa, axis=-1, keepdims=True), (H, 128)), hf == 0)
        return a_block(None, fn)

    def cc_block(j):
        def fn():
            r = _nn(sa_scr[:, j * 512:(j + 1) * 512].astype(BF16), ckv_v[j * 512:(j + 1) * 512, :])
            acc(cc_scr, ..., r, j == 0)
        return a_block(None, fn)

    def ctx_e_block(j, hf):
        def fn():
            cc = (cc_scr[:, j * 128:(j + 1) * 128] / la_scr[...]).astype(BF16)
            tm_scr[:, hf * HB:(hf + 1) * HB] = mask_heads(_nn(cc, r0_scr[:, hf * HB:(hf + 1) * HB]))
        return a_block((wuv_v, sem_w.at[3]) if j == 0 and hf == 0 else None, fn)

    def ctx_m_block(j, hf):
        def fn():
            r = _nn(tm_scr[:, hf * HB:(hf + 1) * HB],
                    wuv_v[j * 4096 + hf * HB:j * 4096 + (hf + 1) * HB, :])
            acc(ctx_scr, ..., r, j == 0 and hf == 0)
        return a_block(None, fn)

    def flat_block():
        for k in range(H):
            cf_scr[:, k * D:(k + 1) * D] = jnp.broadcast_to(ctx_scr[k:k + 1, :], (8, D))

    b_rounds = {SM_ROUND} | {2 * pos + 1 for pos in V_TRIG} | {2 * pos + 1 for pos in K_TRIG}
    free = [r for r in range(NR) if r not in b_rounds and r - 1 not in b_rounds]
    slots = A_SLOTS if A_SLOTS is not None else free[1::2]
    sched = {r: [] for r in range(NR)}

    def grp(fs):
        def f():
            for x in fs:
                x()
        return f

    def place(blocks, after_piece, start, allowed, group=AG):
        g = max(w_global_round(after_piece) + MARGIN, start)
        blocks = [grp(blocks[i:i + group]) for i in range(0, len(blocks), group)]
        for b in blocks:
            while g % NR not in allowed:
                g += 1
            assert g // NR < H - 1
            sched[g % NR].append((g // NR, b))
            g += 1
        return g

    g = place([qa_block(j, hf) for j in range(5) for hf in range(2)], wlo[2] - 1, 0, slots)
    g = place([blk for j in range(4) for blk in (qabs_t_block(j, 0), qabs_t_block(j, 1),
                                                 qabs_c_block(j, 0), qabs_c_block(j, 1))],
              wlo[3] - 1, g, slots)
    g = place([sc_block(j) for j in range(8)]
              + [a_block(None, sma_max), sma_exp(0), sma_exp(1)]
              + [cc_block(j) for j in range(8)], wlo[4] - 1, g, slots)
    g = place([blk for j in range(4) for blk in (ctx_e_block(j, 0), ctx_e_block(j, 1),
                                                 ctx_m_block(j, 0), ctx_m_block(j, 1))]
              + [a_block(None, flat_block)], wlo[5] - 1, g, slots)
    k_rest = 0
    while k_rest < H - WOA_TAIL:
        k1 = min(k_rest + PGRP, H - WOA_TAIL)
        last = wlo[5] + PPH * k1 - 1
        if last >= W_LOOP_END:
            break
        g2 = max(g, w_global_round(last) + MARGIN)
        while g2 % NR not in free:
            g2 += 1
        if g2 // NR >= H - 1:
            break
        sched[g2 % NR].append((g2 // NR, proj_a(k_rest, k1)))
        g = g2 + 1
        k_rest = k1

    PB = 128 // QROWS
    allseq = seq + main
    for i in range(NPRO):
        seq[i]().wait()
        if i + PD < len(allseq):
            allseq[i + PD]().start(priority=P1)
        if i >= NPRO - (DEPTH - PD) and DEPTH > PD:
            allseq[NPRO + PD + (i - (NPRO - (DEPTH - PD)))]().start(priority=P1)
        w_issue(i)
        if i in (0, 1):
            setup_r0(i)
        if i in (2, 3):
            setup_r0t(i - 2)
        if i == 4:
            setup_x()
        if PB - 1 <= i <= NQP and i % PB in (PB - 1, 0):
            qb_part((i - PB + 1) // PB, 0 if i % PB == PB - 1 else 1)
        for p in K_TRIG.get(i - NQP, []):
            qk_part(0, p)

    def body(h, carry):
        for r in range(NR):
            p1_copy(h, r).wait()
            if W_FIRST and r in W_ROUNDS:
                w_issue(W_BASE + h * NWR + W_ROUNDS.index(r))
            dh, r2 = divmod(r + DEPTH, NR)
            lim = H - 1 - dh if r2 % 2 == 0 else H - dh
            if lim >= H - 1:
                p1_copy(h + dh, r2).start(priority=P1)
            else:
                @pl.when(h < lim)
                def _():
                    p1_copy(h + dh, r2).start(priority=P1)
            if not W_FIRST and r in W_ROUNDS:
                w_issue(W_BASE + h * NWR + W_ROUNDS.index(r))
            if r == 0:
                wait_head_rows(wob_v, sem_wob, h)
            if r == SM_ROUND:
                softmax_b()
                proj_b(jnp.maximum(h - 1, 0))
            if r % 2 == 1:
                for p in K_TRIG.get(r // 2, []):
                    qk_part(h + 1, p)
                for p in V_TRIG.get(r // 2, []):
                    pv_part(h, p)
            if sched[r]:
                mask = sum(1 << hs for hs in {hs for hs, _ in sched[r]})

                @pl.when(jnp.bitwise_and(lax.shift_right_logical(jnp.int32(mask), h), 1) == 1)
                def _():
                    for hs, f in sched[r]:
                        pl.when(h == hs)(f)
        return carry

    lax.fori_loop(0, H - 1, body, 0)

    h = H - 1
    issued = set()
    for gidx in range(DEPTH, (H - 1) * NR + DEPTH):
        if gidx // NR == h and gidx % 2 == 1:
            issued.add((gidx % NR) // 2)
    for gidx in range(DEPTH):
        if gidx // NR == h and gidx % 2 == 1:
            issued.add((gidx % NR) // 2)
    pending = [j for j in range(NP) if j not in issued]

    SPLIT = H * D - LASTR

    def rows_copy(lo, hi, sem):
        return pltpu.make_async_copy(woa_hbm.at[pl.ds(lo, hi - lo)], woa_v.at[pl.ds(lo, hi - lo)], sem)

    def start_tail():
        for k in range(H - WOA_TAIL, H):
            rows_copy(k * D, min((k + 1) * D, SPLIT), sem_woa.at[k]).start(priority=P1)
        if LASTR:
            rows_copy(SPLIT, H * D, sem_s.at[0]).start(priority=P1)

    if not pending:
        start_tail()
    wi = W_LOOP_END
    k_next = k_rest
    w_round = {}
    for j in range(NP):
        v_copy(h, VSEQ[j]).wait()
        if pending:
            v_copy(h, VSEQ[pending.pop(0)]).start(priority=P1)
            if not pending:
                start_tail()
        for _ in range(TAIL_W):
            if wi < NW:
                w_issue(wi)
                w_round[wi] = j
                wi += 1
        if j == 0:
            wait_head_rows(wob_v, sem_wob, h)
            softmax_b()
            proj_b(h - 1)
        if j in V_TRIG:
            for p in V_TRIG[j]:
                pv_part(h, p)
        elif j >= 1:
            k1 = k_next
            while (k1 < H - WOA_TAIL and k1 < k_next + PGRP and wlo[5] + PPH * (k1 + 1) - 1 < wi
                   and w_round.get(wlo[5] + PPH * (k1 + 1) - 1, -100) <= j - 4):
                k1 += 1
            if k1 > k_next:
                proj_a(k_next, k1)()
                k_next = k1
    assert wi >= NW
    proj_b(h)
    if k_next < H - WOA_TAIL:
        proj_a(k_next, H - WOA_TAIL)()
    for k in range(H - WOA_TAIL, H):
        lo, hi = k * D, min((k + 1) * D, SPLIT)
        rows_copy(lo, hi, sem_woa.at[k]).wait()
        acca_scr[...] += _nn(cf_scr[:, lo:hi].astype(BF16), woa_v[lo:hi, :])

    g = g_scr[0:1, 0:1]
    part = g * acca_scr[0:1, :] + (1.0 - g) * accb_scr[0:1, :]
    if LASTR and LAST_VPU:
        crow = cf_scr[0:1, H * D - 128:H * D].astype(BF16).astype(F32)
        sel = (lax.broadcasted_iota(jnp.int32, (LASTR, 128), 1)
               == lax.broadcasted_iota(jnp.int32, (LASTR, 128), 0) + (128 - LASTR))
        ccol = jnp.sum(jnp.where(sel, crow, 0.0), axis=1, keepdims=True) * g
        rows_copy(SPLIT, H * D, sem_s.at[0]).wait()
        part = part + jnp.sum(woa_v[SPLIT:H * D, :].astype(F32) * ccol, axis=0, keepdims=True)
    elif LASTR:
        rows_copy(SPLIT, H * D, sem_s.at[0]).wait()
        part = part + g * _nn(cf_scr[:, SPLIT:H * D].astype(BF16), woa_v[SPLIT:H * D, :])[0:1, :]
    o_ref[0] = part.astype(o_ref.dtype)


@jax.jit
def pallas_gated_mix__compressed_kv_cla__gqa_block_cached__decode_kernel(
    A_x, A_c_kv, A_w_q, A_w_uk, A_w_uv, A_w_o, B_x, B_k_cache, B_v_cache, B_wq, B_wo, gate_w,
):
    ckv = A_c_kv.reshape(S, C)
    wqa = A_w_q.reshape(M * H, D)
    wuk = A_w_uk.reshape(C * H, D)
    wuv = A_w_uv.reshape(C * H, D)
    woa = A_w_o.reshape(H * D, M)
    k = B_k_cache.reshape(H, S, D)
    v = B_v_cache.reshape(H, S, D)

    any_spec = pl.BlockSpec(memory_space=pl.ANY)
    return pl.pallas_call(
        _kernel,
        in_specs=[any_spec] * 12,
        out_specs=pl.BlockSpec(memory_space=pltpu.VMEM),
        out_shape=jax.ShapeDtypeStruct((1, 1, M), BF16),
        scratch_shapes=[
            pltpu.VMEM((S, C), BF16),
            pltpu.VMEM((M * H, D), BF16),
            pltpu.VMEM((C * H, D), BF16),
            pltpu.VMEM((C * H, D), BF16),
            pltpu.VMEM((H * D, M), BF16),
            pltpu.VMEM((M, H * D), BF16),
            pltpu.VMEM((H * D, M), BF16),
            pltpu.VMEM((NB, S, D), BF16),
            pltpu.VMEM((NB, S, D), BF16),
            pltpu.VMEM((H, 8, D), F32),
            pltpu.VMEM((8, S), F32),
            pltpu.VMEM((8, S), F32),
            pltpu.VMEM((8, D), F32),
            pltpu.VMEM((8, D), F32),
            pltpu.VMEM((128, 4096), BF16),
            pltpu.VMEM((4096, 128), BF16),
            pltpu.VMEM((8, 4096), F32),
            pltpu.VMEM((H, D), F32),
            pltpu.VMEM((H, 4096), BF16),
            pltpu.VMEM((H, C), F32),
            pltpu.VMEM((H, S), F32),
            pltpu.VMEM((H, 128), F32),
            pltpu.VMEM((H, 128), F32),
            pltpu.VMEM((H, C), F32),
            pltpu.VMEM((H, D), F32),
            pltpu.VMEM((8, H * D), F32),
            pltpu.VMEM((8, M), F32),
            pltpu.VMEM((8, M), F32),
            pltpu.VMEM((8, 128), F32),
            pltpu.VMEM((1, 1, M), BF16),
            pltpu.VMEM((1, 1, M), BF16),
            pltpu.VMEM((M,), BF16),
            pltpu.SemaphoreType.DMA((3,)),
            pltpu.SemaphoreType.DMA((PD,)),
            pltpu.SemaphoreType.DMA((NB * NP,)),
            pltpu.SemaphoreType.DMA((NB * NP,)),
            pltpu.SemaphoreType.DMA((4,)),
            pltpu.SemaphoreType.DMA((32,)),
            pltpu.SemaphoreType.DMA((32,)),
        ],
        compiler_params=pltpu.CompilerParams(vmem_limit_bytes=100 * 1024 * 1024,
                                             disable_bounds_checks=True,
                                             disable_semaphore_checks=True),
    )(A_x, B_x, gate_w, ckv, wqa, wuk, wuv, woa, k, v, B_wq, B_wo)
```

```python
import functools
import jax
import jax.numpy as jnp
from jax import lax
import jax.experimental.pallas as pl
import jax.experimental.pallas.tpu as pltpu

F32 = jnp.float32
BF16 = jnp.bfloat16

H = 32
D = 128
S = 4096
M = 640
C = 512
SCALE = float(D) ** -0.5


PCH = [320] * 10 + [256] + [320] * 2
POFF = [sum(PCH[:i]) for i in range(len(PCH))]
NP = len(PCH)
NR = 2 * NP
PARTS = [(0, 1280), (1280, 2560), (2560, 4096)]
VROT = 4
VSEQ = [(j + VROT) % NP for j in range(NP)]


def _triggers(order):
    trig = {}
    for p, (lo, hi) in enumerate(PARTS):
        need = [j for j in range(NP) if POFF[j] < hi and POFF[j] + PCH[j] > lo]
        trig.setdefault(max(order.index(j) for j in need), []).append(p)
    return trig


K_TRIG = _triggers(list(range(NP)))
V_TRIG = _triggers(VSEQ)
V_ORDER = [p for pos in sorted(V_TRIG) for p in V_TRIG[pos]]
DEPTH = NR
NB = 2
assert DEPTH <= NR * (NB - 1) and DEPTH % 2 == 0
P0, P1 = 0, 1
WOA_TAIL = 4
QROWS = 8
NQP = M // QROWS
PD = 32
NPRO = NQP + NP
W_SKIP = (2, 9, 16, 23)
W_ROUNDS = [r for r in range(NR) if r not in W_SKIP]
NWR = len(W_ROUNDS)
WOP = 32
WQP = 128
WUP = 128
WCP = 32
TAIL_W = 1
SM_ROUND = 1
AG = 2
A_SLOTS = None
MARGIN = 8
PGRP = 3
W_FIRST = 0
LASTR = 128
NSUB = 4
SUBR = LASTR // NSUB


def _nt(a, b):
    return lax.dot_general(a, b, (((1,), (1,)), ((), ())), preferred_element_type=F32)


def _nn(a, b):
    return jnp.dot(a, b, preferred_element_type=F32)


def shr(k, n):
    return k >> n if isinstance(k, int) else lax.shift_right_logical(k, n)


def band(k, n):
    return k & n if isinstance(k, int) else jnp.bitwise_and(k, n)


def _kernel(xa_hbm, xb_hbm, gw_hbm, ckv_hbm, wqa_hbm, wuk_hbm, wuv_hbm, woa_hbm,
            k_hbm, v_hbm, wqb_hbm, wob_hbm,
            o_ref,
            ckv_v, wqa_v, wuk_v, wuv_v, woa_v, wqb_v, wob_v,
            k_buf, v_buf, q_scr, s_scr, p_scr, l_scr, o_scr, r0_scr, r0t_scr, xe_scr,
            qa_scr, tm_scr, qabs_scr, sa_scr, ma_scr, la_scr, cc_scr, ctx_scr, cf_scr,
            acca_scr, accb_scr, g_scr, cb_scr, xa_v, xb_v, gw_v,
            sem_s, sem_t, sem_q, sem_k, sem_v, sem_w, sem_wob, sem_woa):
    def k_copy(h, j):
        b = band(h, NB - 1)
        return pltpu.make_async_copy(k_hbm.at[h, pl.ds(POFF[j], PCH[j])],
                                     k_buf.at[b, pl.ds(POFF[j], PCH[j])], sem_k.at[b * NP + j])

    def v_copy(h, j):
        b = band(h, NB - 1)
        return pltpu.make_async_copy(v_hbm.at[h, pl.ds(POFF[j], PCH[j])],
                                     v_buf.at[b, pl.ds(POFF[j], PCH[j])], sem_v.at[b * NP + j])

    def row_piece(src, dst, k, rows, sem):
        return pltpu.make_async_copy(src.at[pl.ds(k * rows, rows)], dst.at[pl.ds(k * rows, rows)], sem)

    def wq_copy(i):
        return row_piece(wqb_hbm, wqb_v, i, QROWS, sem_q.at[i % PD])

    PPH = D // WOP
    SH = PPH.bit_length() - 1
    wtab = [
        (H * PPH, lambda k: row_piece(wob_hbm, wob_v, k, WOP, sem_wob.at[shr(k, SH)])),
        (M * H // WQP, lambda k: row_piece(wqa_hbm, wqa_v, k, WQP, sem_w.at[0])),
        (C * H // WUP, lambda k: row_piece(wuk_hbm, wuk_v, k, WUP, sem_w.at[1])),
        (S // WCP, lambda k: row_piece(ckv_hbm, ckv_v, k, WCP, sem_w.at[2])),
        (C * H // WUP, lambda k: row_piece(wuv_hbm, wuv_v, k, WUP, sem_w.at[3])),
        ((H - WOA_TAIL) * PPH, lambda k: row_piece(woa_hbm, woa_v, k, WOP, sem_woa.at[shr(k, SH)])),
    ]
    wlo = [sum(n for n, _ in wtab[:a]) for a in range(len(wtab) + 1)]
    NW = wlo[-1]
    W_BASE = NPRO
    W_LOOP_END = W_BASE + (H - 1) * NWR
    assert W_LOOP_END + NP * TAIL_W >= NW, (W_LOOP_END + NP * TAIL_W, NW)

    def w_global_round(i):
        k = i - W_BASE
        if k < 0:
            return -1
        return (k // NWR) * NR + W_ROUNDS[k % NWR]

    def w_issue(i):
        if isinstance(i, int):
            for a, (n, f) in enumerate(wtab):
                if wlo[a] <= i < wlo[a + 1]:
                    f(i - wlo[a]).start(priority=P0)
            return
        for a, (n, f) in enumerate(wtab):
            @pl.when(jnp.logical_and(i >= wlo[a], i < wlo[a + 1]))
            def _():
                f(i - wlo[a]).start(priority=P0)

    def wait_all(buf, sem):
        pltpu.make_async_copy(buf, buf, sem).wait()

    def wait_head_rows(w_v, sem, k):
        off = k * D if isinstance(k, int) else pl.multiple_of(k * D, D)
        blk = w_v.at[pl.ds(off, D)]
        pltpu.make_async_copy(blk, blk, sem.at[k]).wait()

    def p1_copy(h, r):
        return k_copy(h + 1, r // 2) if r % 2 == 0 else v_copy(h, VSEQ[r // 2])

    small = [pltpu.make_async_copy(xb_hbm, xb_v, sem_s.at[0]),
             pltpu.make_async_copy(xa_hbm, xa_v, sem_s.at[1]),
             pltpu.make_async_copy(gw_hbm, gw_v, sem_s.at[2])]
    seq = [functools.partial(wq_copy, i) for i in range(NQP)]
    seq += [functools.partial(k_copy, 0, j) for j in range(NP)]
    main = [functools.partial(p1_copy, g // NR, g % NR) for g in range(DEPTH)]
    for i in range(PD):
        seq[i]().start(priority=P1)
    for c in small:
        c.start(priority=P0)

    def hmask128():
        return (jnp.bitwise_and(lax.broadcasted_iota(jnp.int32, (H, 128), 1), H - 1)
                == lax.broadcasted_iota(jnp.int32, (H, 128), 0))

    def mask_heads(t):
        m = hmask128()
        return jnp.concatenate(
            [jnp.where(m, t[:, b * 128:(b + 1) * 128], 0.0) for b in range(t.shape[1] // 128)],
            axis=1).astype(BF16)

    def setup_r0(hf):
        cols = lax.broadcasted_iota(jnp.int32, (128, 2048), 1) + hf * 2048
        r0_scr[:, hf * 2048:(hf + 1) * 2048] = (
            lax.shift_right_logical(cols, 5)
            == lax.broadcasted_iota(jnp.int32, (128, 2048), 0)).astype(F32).astype(BF16)

    def setup_r0t(hf):
        rows = lax.broadcasted_iota(jnp.int32, (2048, 128), 0) + hf * 2048
        r0t_scr[hf * 2048:(hf + 1) * 2048, :] = (
            lax.shift_right_logical(rows, 5)
            == lax.broadcasted_iota(jnp.int32, (2048, 128), 1)).astype(F32).astype(BF16)

    def setup_x():
        acca_scr[...] = jnp.zeros((8, M), F32)
        accb_scr[...] = jnp.zeros((8, M), F32)
        o_scr[...] = jnp.zeros((8, D), F32)
        for c in small:
            c.wait()
        xa = xa_v[0].astype(F32)
        x8 = jnp.concatenate([xa[:, j * 128:(j + 1) * 128] for j in range(M // 128)]
                             + [jnp.zeros((3, 128), F32)], axis=0)
        xe_scr[...] = _nn(x8.astype(BF16), r0_scr[...])
        gw = gw_v[...].astype(F32).reshape(1, M)
        g = jax.nn.sigmoid(jnp.sum(xa * gw, axis=-1, keepdims=True))
        g_scr[...] = jnp.broadcast_to(g, (8, 128))

    def qb_part(blk, half):
        xb8 = jnp.broadcast_to(xb_v[0][:, blk * 128:(blk + 1) * 128].astype(F32), (8, 128)).astype(BF16)
        qb = _nn(xb8, wqb_v[blk * 128:(blk + 1) * 128, half * 2048:(half + 1) * 2048])
        for hh in range(16):
            if blk == 0:
                q_scr[half * 16 + hh] = qb[:, hh * D:(hh + 1) * D]
            else:
                q_scr[half * 16 + hh] += qb[:, hh * D:(hh + 1) * D]

    def qk_part(hn, part):
        lo, hi = PARTS[part]
        q = q_scr[hn].astype(BF16)
        s_scr[:, lo:hi] = _nt(q, k_buf[band(hn, NB - 1), lo:hi, :])

    def softmax_b():
        s = s_scr[...] * SCALE
        p = jnp.exp(s - jnp.max(s, axis=-1, keepdims=True))
        p_scr[...] = p
        l_scr[...] = jnp.broadcast_to(jnp.sum(p, axis=-1, keepdims=True), (8, D))

    def pv_part(h, part):
        lo, hi = PARTS[part]
        r = _nn(p_scr[:, lo:hi].astype(BF16), v_buf[band(h, NB - 1), lo:hi, :])
        if part == V_ORDER[0]:
            o_scr[...] = r
        elif part != V_ORDER[-1]:
            o_scr[...] += r
        else:
            o_scr[...] = (o_scr[...] + r) / l_scr[...]

    def proj_b(h):
        off = h * D if isinstance(h, int) else pl.multiple_of(h * D, D)
        accb_scr[...] += _nn(o_scr[...].astype(BF16), wob_v[pl.ds(off, D), :])

    def proj_a(k0, k1):
        def f():
            for k in range(k0, k1):
                wait_head_rows(woa_v, sem_woa, k)
            acca_scr[...] += _nn(cf_scr[:, k0 * D:k1 * D].astype(BF16), woa_v[k0 * D:k1 * D, :])
        return f

    HB = 2048

    def a_block(wait, fn):
        def f():
            if wait is not None:
                wait_all(*wait)
            fn()
        return f

    def acc(ref, idx, r, first):
        if first:
            ref[idx] = r
        else:
            ref[idx] += r

    def qa_block(j, hf):
        def fn():
            xsel = mask_heads(jnp.broadcast_to(xe_scr[j:j + 1, hf * HB:(hf + 1) * HB], (H, HB)))
            r = _nn(xsel, wqa_v[j * 4096 + hf * HB:j * 4096 + (hf + 1) * HB, :])
            acc(qa_scr, ..., r, j == 0 and hf == 0)
        return a_block((wqa_v, sem_w.at[0]) if j == 0 and hf == 0 else None, fn)

    def qabs_t_block(j, hf):
        def fn():
            t = _nt(qa_scr[...].astype(BF16), wuk_v[j * 4096 + hf * HB:j * 4096 + (hf + 1) * HB, :])
            tm_scr[:, hf * HB:(hf + 1) * HB] = mask_heads(t)
        return a_block((wuk_v, sem_w.at[1]) if j == 0 and hf == 0 else None, fn)

    def qabs_c_block(j, hf):
        def fn():
            r = _nn(tm_scr[:, hf * HB:(hf + 1) * HB], r0t_scr[hf * HB:(hf + 1) * HB, :])
            acc(qabs_scr, (slice(None), slice(j * 128, (j + 1) * 128)), r, hf == 0)
        return a_block(None, fn)

    def sc_block(j):
        def fn():
            sa_scr[:, j * 512:(j + 1) * 512] = _nt(qabs_scr[...].astype(BF16),
                                                   ckv_v[j * 512:(j + 1) * 512, :]) * SCALE
        return a_block((ckv_v, sem_w.at[2]) if j == 0 else None, fn)

    def sma_max():
        ma_scr[...] = jnp.broadcast_to(jnp.max(sa_scr[...], axis=-1, keepdims=True), (H, 128))

    def sma_exp(hf):
        def fn():
            pa = jnp.exp(sa_scr[:, hf * HB:(hf + 1) * HB] - ma_scr[:, 0:1])
            sa_scr[:, hf * HB:(hf + 1) * HB] = pa
            acc(la_scr, ..., jnp.broadcast_to(jnp.sum(pa, axis=-1, keepdims=True), (H, 128)), hf == 0)
        return a_block(None, fn)

    def cc_block(j):
        def fn():
            r = _nn(sa_scr[:, j * 512:(j + 1) * 512].astype(BF16), ckv_v[j * 512:(j + 1) * 512, :])
            acc(cc_scr, ..., r, j == 0)
        return a_block(None, fn)

    def ctx_e_block(j, hf):
        def fn():
            cc = (cc_scr[:, j * 128:(j + 1) * 128] / la_scr[...]).astype(BF16)
            tm_scr[:, hf * HB:(hf + 1) * HB] = mask_heads(_nn(cc, r0_scr[:, hf * HB:(hf + 1) * HB]))
        return a_block((wuv_v, sem_w.at[3]) if j == 0 and hf == 0 else None, fn)

    def ctx_m_block(j, hf):
        def fn():
            r = _nn(tm_scr[:, hf * HB:(hf + 1) * HB],
                    wuv_v[j * 4096 + hf * HB:j * 4096 + (hf + 1) * HB, :])
            acc(ctx_scr, ..., r, j == 0 and hf == 0)
        return a_block(None, fn)

    def flat_block():
        for k in range(H):
            cf_scr[:, k * D:(k + 1) * D] = jnp.broadcast_to(ctx_scr[k:k + 1, :], (8, D))
        if LASTR:
            crow = ctx_scr[H - 1:H, :].astype(BF16).astype(F32)
            sel = (lax.broadcasted_iota(jnp.int32, (LASTR, 128), 1)
                   == lax.broadcasted_iota(jnp.int32, (LASTR, 128), 0) + (128 - LASTR))
            ccol = jnp.sum(jnp.where(sel, crow, 0.0), axis=1, keepdims=True) * g_scr[0:1, 0:1]
            cb_scr[0:LASTR, :] = jnp.broadcast_to(ccol, (LASTR, 128))

    b_rounds = {SM_ROUND} | {2 * pos + 1 for pos in V_TRIG} | {2 * pos + 1 for pos in K_TRIG}
    free = [r for r in range(NR) if r not in b_rounds and r - 1 not in b_rounds]
    slots = A_SLOTS if A_SLOTS is not None else free[1::2]
    sched = {r: [] for r in range(NR)}

    def grp(fs):
        def f():
            for x in fs:
                x()
        return f

    def place(blocks, after_piece, start, allowed, group=AG):
        g = max(w_global_round(after_piece) + MARGIN, start)
        blocks = [grp(blocks[i:i + group]) for i in range(0, len(blocks), group)]
        for b in blocks:
            while g % NR not in allowed:
                g += 1
            assert g // NR < H - 1
            sched[g % NR].append((g // NR, b))
            g += 1
        return g

    g = place([qa_block(j, hf) for j in range(5) for hf in range(2)], wlo[2] - 1, 0, slots)
    g = place([blk for j in range(4) for blk in (qabs_t_block(j, 0), qabs_t_block(j, 1),
                                                 qabs_c_block(j, 0), qabs_c_block(j, 1))],
              wlo[3] - 1, g, slots)
    g = place([sc_block(j) for j in range(8)]
              + [a_block(None, sma_max), sma_exp(0), sma_exp(1)]
              + [cc_block(j) for j in range(8)], wlo[4] - 1, g, slots)
    g = place([blk for j in range(4) for blk in (ctx_e_block(j, 0), ctx_e_block(j, 1),
                                                 ctx_m_block(j, 0), ctx_m_block(j, 1))]
              + [a_block(None, flat_block)], wlo[5] - 1, g, slots)
    k_rest = 0
    while k_rest < H - WOA_TAIL:
        k1 = min(k_rest + PGRP, H - WOA_TAIL)
        last = wlo[5] + PPH * k1 - 1
        if last >= W_LOOP_END:
            break
        g2 = max(g, w_global_round(last) + MARGIN)
        while g2 % NR not in free:
            g2 += 1
        if g2 // NR >= H - 1:
            break
        sched[g2 % NR].append((g2 // NR, proj_a(k_rest, k1)))
        g = g2 + 1
        k_rest = k1

    PB = 128 // QROWS
    allseq = seq + main
    for i in range(NPRO):
        seq[i]().wait()
        if i + PD < len(allseq):
            allseq[i + PD]().start(priority=P1)
        if i >= NPRO - (DEPTH - PD) and DEPTH > PD:
            allseq[NPRO + PD + (i - (NPRO - (DEPTH - PD)))]().start(priority=P1)
        w_issue(i)
        if i in (0, 1):
            setup_r0(i)
        if i in (2, 3):
            setup_r0t(i - 2)
        if i == 4:
            setup_x()
        if PB - 1 <= i <= NQP and i % PB in (PB - 1, 0):
            qb_part((i - PB + 1) // PB, 0 if i % PB == PB - 1 else 1)
        for p in K_TRIG.get(i - NQP, []):
            qk_part(0, p)

    def body(h, carry):
        for r in range(NR):
            p1_copy(h, r).wait()
            if W_FIRST and r in W_ROUNDS:
                w_issue(W_BASE + h * NWR + W_ROUNDS.index(r))
            dh, r2 = divmod(r + DEPTH, NR)
            lim = H - 1 - dh if r2 % 2 == 0 else H - dh
            if lim >= H - 1:
                p1_copy(h + dh, r2).start(priority=P1)
            else:
                @pl.when(h < lim)
                def _():
                    p1_copy(h + dh, r2).start(priority=P1)
            if not W_FIRST and r in W_ROUNDS:
                w_issue(W_BASE + h * NWR + W_ROUNDS.index(r))
            if r == 0:
                wait_head_rows(wob_v, sem_wob, h)
            if r == SM_ROUND:
                softmax_b()
                proj_b(jnp.maximum(h - 1, 0))
            if r % 2 == 1:
                for p in K_TRIG.get(r // 2, []):
                    qk_part(h + 1, p)
                for p in V_TRIG.get(r // 2, []):
                    pv_part(h, p)
            if sched[r]:
                mask = sum(1 << hs for hs in {hs for hs, _ in sched[r]})

                @pl.when(jnp.bitwise_and(lax.shift_right_logical(jnp.int32(mask), h), 1) == 1)
                def _():
                    for hs, f in sched[r]:
                        pl.when(h == hs)(f)
        return carry

    lax.fori_loop(0, H - 1, body, 0)

    h = H - 1
    issued = set()
    for gidx in range(DEPTH, (H - 1) * NR + DEPTH):
        if gidx // NR == h and gidx % 2 == 1:
            issued.add((gidx % NR) // 2)
    for gidx in range(DEPTH):
        if gidx // NR == h and gidx % 2 == 1:
            issued.add((gidx % NR) // 2)
    pending = [j for j in range(NP) if j not in issued]

    SPLIT = H * D - LASTR

    def rows_copy(lo, hi, sem):
        return pltpu.make_async_copy(woa_hbm.at[pl.ds(lo, hi - lo)], woa_v.at[pl.ds(lo, hi - lo)], sem)

    def start_tail():
        for k in range(H - WOA_TAIL, H):
            if min((k + 1) * D, SPLIT) > k * D:
                rows_copy(k * D, min((k + 1) * D, SPLIT), sem_woa.at[k]).start(priority=P1)
        for u in range(NSUB if LASTR else 0):
            rows_copy(SPLIT + u * SUBR, SPLIT + (u + 1) * SUBR, sem_t.at[u]).start(priority=P1)

    if not pending:
        start_tail()
    wi = W_LOOP_END
    k_next = k_rest
    w_round = {}
    for j in range(NP):
        v_copy(h, VSEQ[j]).wait()
        if pending:
            v_copy(h, VSEQ[pending.pop(0)]).start(priority=P1)
            if not pending:
                start_tail()
        for _ in range(TAIL_W):
            if wi < NW:
                w_issue(wi)
                w_round[wi] = j
                wi += 1
        if j == 0:
            wait_head_rows(wob_v, sem_wob, h)
            softmax_b()
            proj_b(h - 1)
        if j in V_TRIG:
            for p in V_TRIG[j]:
                pv_part(h, p)
        elif j >= 1:
            k1 = k_next
            while (k1 < H - WOA_TAIL and k1 < k_next + PGRP and wlo[5] + PPH * (k1 + 1) - 1 < wi
                   and w_round.get(wlo[5] + PPH * (k1 + 1) - 1, -100) <= j - 4):
                k1 += 1
            if k1 > k_next:
                proj_a(k_next, k1)()
                k_next = k1
    assert wi >= NW
    proj_b(h)
    if k_next < H - WOA_TAIL:
        proj_a(k_next, H - WOA_TAIL)()
    for k in range(H - WOA_TAIL, H):
        lo, hi = k * D, min((k + 1) * D, SPLIT)
        if hi > lo:
            rows_copy(lo, hi, sem_woa.at[k]).wait()
            acca_scr[...] += _nn(cf_scr[:, lo:hi].astype(BF16), woa_v[lo:hi, :])

    g = g_scr[0:1, 0:1]
    part = g * acca_scr[0:1, :] + (1.0 - g) * accb_scr[0:1, :]
    if LASTR:
        accv = jnp.zeros((8, M), F32)
        for u in range(NSUB):
            lo = SPLIT + u * SUBR
            rows_copy(lo, lo + SUBR, sem_t.at[u]).wait()
            w = woa_v[lo:lo + SUBR, :].astype(F32)
            c = cb_scr[u * SUBR:(u + 1) * SUBR, :]
            prod = w * jnp.concatenate([c] * (M // 128), axis=1)
            for t in range(SUBR // 8):
                accv = accv + prod[t * 8:(t + 1) * 8, :]
        part = part + jnp.sum(accv, axis=0, keepdims=True)
    o_ref[0] = part.astype(o_ref.dtype)


@jax.jit
def pallas_gated_mix__compressed_kv_cla__gqa_block_cached__decode_kernel(
    A_x, A_c_kv, A_w_q, A_w_uk, A_w_uv, A_w_o, B_x, B_k_cache, B_v_cache, B_wq, B_wo, gate_w,
):
    ckv = A_c_kv.reshape(S, C)
    wqa = A_w_q.reshape(M * H, D)
    wuk = A_w_uk.reshape(C * H, D)
    wuv = A_w_uv.reshape(C * H, D)
    woa = A_w_o.reshape(H * D, M)
    k = B_k_cache.reshape(H, S, D)
    v = B_v_cache.reshape(H, S, D)

    any_spec = pl.BlockSpec(memory_space=pl.ANY)
    return pl.pallas_call(
        _kernel,
        in_specs=[any_spec] * 12,
        out_specs=pl.BlockSpec(memory_space=pltpu.VMEM),
        out_shape=jax.ShapeDtypeStruct((1, 1, M), BF16),
        scratch_shapes=[
            pltpu.VMEM((S, C), BF16),
            pltpu.VMEM((M * H, D), BF16),
            pltpu.VMEM((C * H, D), BF16),
            pltpu.VMEM((C * H, D), BF16),
            pltpu.VMEM((H * D, M), BF16),
            pltpu.VMEM((M, H * D), BF16),
            pltpu.VMEM((H * D, M), BF16),
            pltpu.VMEM((NB, S, D), BF16),
            pltpu.VMEM((NB, S, D), BF16),
            pltpu.VMEM((H, 8, D), F32),
            pltpu.VMEM((8, S), F32),
            pltpu.VMEM((8, S), F32),
            pltpu.VMEM((8, D), F32),
            pltpu.VMEM((8, D), F32),
            pltpu.VMEM((128, 4096), BF16),
            pltpu.VMEM((4096, 128), BF16),
            pltpu.VMEM((8, 4096), F32),
            pltpu.VMEM((H, D), F32),
            pltpu.VMEM((H, 4096), BF16),
            pltpu.VMEM((H, C), F32),
            pltpu.VMEM((H, S), F32),
            pltpu.VMEM((H, 128), F32),
            pltpu.VMEM((H, 128), F32),
            pltpu.VMEM((H, C), F32),
            pltpu.VMEM((H, D), F32),
            pltpu.VMEM((8, H * D), F32),
            pltpu.VMEM((8, M), F32),
            pltpu.VMEM((8, M), F32),
            pltpu.VMEM((8, 128), F32),
            pltpu.VMEM((128, 128), F32),
            pltpu.VMEM((1, 1, M), BF16),
            pltpu.VMEM((1, 1, M), BF16),
            pltpu.VMEM((M,), BF16),
            pltpu.SemaphoreType.DMA((3,)),
            pltpu.SemaphoreType.DMA((NSUB,)),
            pltpu.SemaphoreType.DMA((PD,)),
            pltpu.SemaphoreType.DMA((NB * NP,)),
            pltpu.SemaphoreType.DMA((NB * NP,)),
            pltpu.SemaphoreType.DMA((4,)),
            pltpu.SemaphoreType.DMA((32,)),
            pltpu.SemaphoreType.DMA((32,)),
        ],
        compiler_params=pltpu.CompilerParams(vmem_limit_bytes=100 * 1024 * 1024,
                                             disable_bounds_checks=True,
                                             disable_semaphore_checks=True),
    )(A_x, B_x, gate_w, ckv, wqa, wuk, wuv, woa, k, v, B_wq, B_wo)
```

```python
import functools
import jax
import jax.numpy as jnp
from jax import lax
import jax.experimental.pallas as pl
import jax.experimental.pallas.tpu as pltpu

F32 = jnp.float32
BF16 = jnp.bfloat16

H = 32
D = 128
S = 4096
M = 640
C = 512
SCALE = float(D) ** -0.5


PCH = [320] * 10 + [256] + [320] * 2
POFF = [sum(PCH[:i]) for i in range(len(PCH))]
NP = len(PCH)
NR = 2 * NP
PARTS = [(0, 1280), (1280, 2560), (2560, 4096)]
VROT = 4
VSEQ = [(j + VROT) % NP for j in range(NP)]


def _triggers(order):
    trig = {}
    for p, (lo, hi) in enumerate(PARTS):
        need = [j for j in range(NP) if POFF[j] < hi and POFF[j] + PCH[j] > lo]
        trig.setdefault(max(order.index(j) for j in need), []).append(p)
    return trig


K_TRIG = _triggers(list(range(NP)))
V_TRIG = _triggers(VSEQ)
V_ORDER = [p for pos in sorted(V_TRIG) for p in V_TRIG[pos]]
DEPTH = NR
NB = 2
assert DEPTH <= NR * (NB - 1) and DEPTH % 2 == 0
P0, P1 = 0, 1
WOA_TAIL = 4
QROWS = 8
NQP = M // QROWS
PD = 32
NPRO = NQP + NP
W_SKIP = (2, 9, 16, 23)
W_ROUNDS = [r for r in range(NR) if r not in W_SKIP]
NWR = len(W_ROUNDS)
WOP = 32
WQP = 128
WUP = 128
WCP = 32
TAIL_W = 1
SM_ROUND = 1
AG = 2
A_SLOTS = None
MARGIN = 8
PGRP = 3
W_FIRST = 0
LASTR = 128
NSUB = 4
SUBR = LASTR // NSUB


def _nt(a, b):
    return lax.dot_general(a, b, (((1,), (1,)), ((), ())), preferred_element_type=F32)


def _nn(a, b):
    return jnp.dot(a, b, preferred_element_type=F32)


def shr(k, n):
    return k >> n if isinstance(k, int) else lax.shift_right_logical(k, n)


def band(k, n):
    return k & n if isinstance(k, int) else jnp.bitwise_and(k, n)


def _kernel(xa_hbm, gw_hbm, ckv_hbm, wqa_hbm, wuk_hbm, wuv_hbm, woa_hbm,
            k_hbm, v_hbm, wqb_hbm, wob_hbm,
            o_ref,
            ckv_v, wqa_v, wuk_v, wuv_v, woa_v, wqb_v, wob_v,
            k_buf, v_buf, q_scr, s_scr, p_scr, l_scr, o_scr, r0_scr, r0t_scr, xe_scr,
            qa_scr, tm_scr, qabs_scr, sa_scr, ma_scr, la_scr, cc_scr, ctx_scr, cf_scr,
            acca_scr, accb_scr, g_scr, cb_scr, xa_v, gw_v,
            sem_s, sem_t, sem_q, sem_k, sem_v, sem_w, sem_wob, sem_woa):
    def k_copy(h, j):
        b = band(h, NB - 1)
        return pltpu.make_async_copy(k_hbm.at[h, pl.ds(POFF[j], PCH[j])],
                                     k_buf.at[b, pl.ds(POFF[j], PCH[j])], sem_k.at[b * NP + j])

    def v_copy(h, j):
        b = band(h, NB - 1)
        return pltpu.make_async_copy(v_hbm.at[h, pl.ds(POFF[j], PCH[j])],
                                     v_buf.at[b, pl.ds(POFF[j], PCH[j])], sem_v.at[b * NP + j])

    def row_piece(src, dst, k, rows, sem):
        return pltpu.make_async_copy(src.at[pl.ds(k * rows, rows)], dst.at[pl.ds(k * rows, rows)], sem)

    def wq_copy(i):
        return row_piece(wqb_hbm, wqb_v, i, QROWS, sem_q.at[i % PD])

    PPH = D // WOP
    SH = PPH.bit_length() - 1
    wtab = [
        (H * PPH, lambda k: row_piece(wob_hbm, wob_v, k, WOP, sem_wob.at[shr(k, SH)])),
        (M * H // WQP, lambda k: row_piece(wqa_hbm, wqa_v, k, WQP, sem_w.at[0])),
        (C * H // WUP, lambda k: row_piece(wuk_hbm, wuk_v, k, WUP, sem_w.at[1])),
        (S // WCP, lambda k: row_piece(ckv_hbm, ckv_v, k, WCP, sem_w.at[2])),
        (C * H // WUP, lambda k: row_piece(wuv_hbm, wuv_v, k, WUP, sem_w.at[3])),
        ((H - WOA_TAIL) * PPH, lambda k: row_piece(woa_hbm, woa_v, k, WOP, sem_woa.at[shr(k, SH)])),
    ]
    wlo = [sum(n for n, _ in wtab[:a]) for a in range(len(wtab) + 1)]
    NW = wlo[-1]
    W_BASE = NPRO
    W_LOOP_END = W_BASE + (H - 1) * NWR
    assert W_LOOP_END + NP * TAIL_W >= NW, (W_LOOP_END + NP * TAIL_W, NW)

    def w_global_round(i):
        k = i - W_BASE
        if k < 0:
            return -1
        return (k // NWR) * NR + W_ROUNDS[k % NWR]

    def w_issue(i):
        if isinstance(i, int):
            for a, (n, f) in enumerate(wtab):
                if wlo[a] <= i < wlo[a + 1]:
                    f(i - wlo[a]).start(priority=P0)
            return
        for a, (n, f) in enumerate(wtab):
            @pl.when(jnp.logical_and(i >= wlo[a], i < wlo[a + 1]))
            def _():
                f(i - wlo[a]).start(priority=P0)

    def wait_all(buf, sem):
        pltpu.make_async_copy(buf, buf, sem).wait()

    def wait_head_rows(w_v, sem, k):
        off = k * D if isinstance(k, int) else pl.multiple_of(k * D, D)
        blk = w_v.at[pl.ds(off, D)]
        pltpu.make_async_copy(blk, blk, sem.at[k]).wait()

    def p1_copy(h, r):
        return k_copy(h + 1, r // 2) if r % 2 == 0 else v_copy(h, VSEQ[r // 2])

    small = [pltpu.make_async_copy(xa_hbm, xa_v, sem_s.at[0]),
             pltpu.make_async_copy(gw_hbm, gw_v, sem_s.at[1])]
    seq = [functools.partial(wq_copy, i) for i in range(NQP)]
    seq += [functools.partial(k_copy, 0, j) for j in range(NP)]
    main = [functools.partial(p1_copy, g // NR, g % NR) for g in range(DEPTH)]
    for i in range(PD):
        seq[i]().start(priority=P1)
    for c in small:
        c.start(priority=P0)

    def hmask128():
        return (jnp.bitwise_and(lax.broadcasted_iota(jnp.int32, (H, 128), 1), H - 1)
                == lax.broadcasted_iota(jnp.int32, (H, 128), 0))

    def mask_heads(t):
        m = hmask128()
        return jnp.concatenate(
            [jnp.where(m, t[:, b * 128:(b + 1) * 128], 0.0) for b in range(t.shape[1] // 128)],
            axis=1).astype(BF16)

    def setup_r0(hf):
        cols = lax.broadcasted_iota(jnp.int32, (128, 2048), 1) + hf * 2048
        r0_scr[:, hf * 2048:(hf + 1) * 2048] = (
            lax.shift_right_logical(cols, 5)
            == lax.broadcasted_iota(jnp.int32, (128, 2048), 0)).astype(F32).astype(BF16)

    def setup_r0t(hf):
        rows = lax.broadcasted_iota(jnp.int32, (2048, 128), 0) + hf * 2048
        r0t_scr[hf * 2048:(hf + 1) * 2048, :] = (
            lax.shift_right_logical(rows, 5)
            == lax.broadcasted_iota(jnp.int32, (2048, 128), 1)).astype(F32).astype(BF16)

    def setup_x():
        acca_scr[...] = jnp.zeros((8, M), F32)
        accb_scr[...] = jnp.zeros((8, M), F32)
        o_scr[...] = jnp.zeros((8, D), F32)
        for c in small:
            c.wait()
        xa = xa_v[0].astype(F32)
        x8 = jnp.concatenate([xa[:, j * 128:(j + 1) * 128] for j in range(M // 128)]
                             + [jnp.zeros((3, 128), F32)], axis=0)
        xe_scr[...] = _nn(x8.astype(BF16), r0_scr[...])
        gw = gw_v[...].astype(F32).reshape(1, M)
        g = jax.nn.sigmoid(jnp.sum(xa * gw, axis=-1, keepdims=True))
        g_scr[...] = jnp.broadcast_to(g, (8, 128))

    def qb_part(blk, half):
        xb8 = jnp.broadcast_to(xa_v[0][:, blk * 128:(blk + 1) * 128].astype(F32), (8, 128)).astype(BF16)
        qb = _nn(xb8, wqb_v[blk * 128:(blk + 1) * 128, half * 2048:(half + 1) * 2048])
        for hh in range(16):
            if blk == 0:
                q_scr[half * 16 + hh] = qb[:, hh * D:(hh + 1) * D]
            else:
                q_scr[half * 16 + hh] += qb[:, hh * D:(hh + 1) * D]

    def qk_part(hn, part):
        lo, hi = PARTS[part]
        q = q_scr[hn].astype(BF16)
        s_scr[:, lo:hi] = _nt(q, k_buf[band(hn, NB - 1), lo:hi, :])

    def softmax_b():
        s = s_scr[...] * SCALE
        p = jnp.exp(s - jnp.max(s, axis=-1, keepdims=True))
        p_scr[...] = p
        l_scr[...] = jnp.broadcast_to(jnp.sum(p, axis=-1, keepdims=True), (8, D))

    def pv_part(h, part):
        lo, hi = PARTS[part]
        r = _nn(p_scr[:, lo:hi].astype(BF16), v_buf[band(h, NB - 1), lo:hi, :])
        if part == V_ORDER[0]:
            o_scr[...] = r
        elif part != V_ORDER[-1]:
            o_scr[...] += r
        else:
            o_scr[...] = (o_scr[...] + r) / l_scr[...]

    def proj_b(h):
        off = h * D if isinstance(h, int) else pl.multiple_of(h * D, D)
        accb_scr[...] += _nn(o_scr[...].astype(BF16), wob_v[pl.ds(off, D), :])

    def proj_a(k0, k1):
        def f():
            for k in range(k0, k1):
                wait_head_rows(woa_v, sem_woa, k)
            acca_scr[...] += _nn(cf_scr[:, k0 * D:k1 * D].astype(BF16), woa_v[k0 * D:k1 * D, :])
        return f

    HB = 2048

    def a_block(wait, fn):
        def f():
            if wait is not None:
                wait_all(*wait)
            fn()
        return f

    def acc(ref, idx, r, first):
        if first:
            ref[idx] = r
        else:
            ref[idx] += r

    def qa_block(j, hf):
        def fn():
            xsel = mask_heads(jnp.broadcast_to(xe_scr[j:j + 1, hf * HB:(hf + 1) * HB], (H, HB)))
            r = _nn(xsel, wqa_v[j * 4096 + hf * HB:j * 4096 + (hf + 1) * HB, :])
            acc(qa_scr, ..., r, j == 0 and hf == 0)
        return a_block((wqa_v, sem_w.at[0]) if j == 0 and hf == 0 else None, fn)

    def qabs_t_block(j, hf):
        def fn():
            t = _nt(qa_scr[...].astype(BF16), wuk_v[j * 4096 + hf * HB:j * 4096 + (hf + 1) * HB, :])
            tm_scr[:, hf * HB:(hf + 1) * HB] = mask_heads(t)
        return a_block((wuk_v, sem_w.at[1]) if j == 0 and hf == 0 else None, fn)

    def qabs_c_block(j, hf):
        def fn():
            r = _nn(tm_scr[:, hf * HB:(hf + 1) * HB], r0t_scr[hf * HB:(hf + 1) * HB, :])
            acc(qabs_scr, (slice(None), slice(j * 128, (j + 1) * 128)), r, hf == 0)
        return a_block(None, fn)

    def sc_block(j):
        def fn():
            sa_scr[:, j * 512:(j + 1) * 512] = _nt(qabs_scr[...].astype(BF16),
                                                   ckv_v[j * 512:(j + 1) * 512, :]) * SCALE
        return a_block((ckv_v, sem_w.at[2]) if j == 0 else None, fn)

    def sma_max():
        ma_scr[...] = jnp.broadcast_to(jnp.max(sa_scr[...], axis=-1, keepdims=True), (H, 128))

    def sma_exp(hf):
        def fn():
            pa = jnp.exp(sa_scr[:, hf * HB:(hf + 1) * HB] - ma_scr[:, 0:1])
            sa_scr[:, hf * HB:(hf + 1) * HB] = pa
            acc(la_scr, ..., jnp.broadcast_to(jnp.sum(pa, axis=-1, keepdims=True), (H, 128)), hf == 0)
        return a_block(None, fn)

    def cc_block(j):
        def fn():
            r = _nn(sa_scr[:, j * 512:(j + 1) * 512].astype(BF16), ckv_v[j * 512:(j + 1) * 512, :])
            acc(cc_scr, ..., r, j == 0)
        return a_block(None, fn)

    def ctx_e_block(j, hf):
        def fn():
            cc = (cc_scr[:, j * 128:(j + 1) * 128] / la_scr[...]).astype(BF16)
            tm_scr[:, hf * HB:(hf + 1) * HB] = mask_heads(_nn(cc, r0_scr[:, hf * HB:(hf + 1) * HB]))
        return a_block((wuv_v, sem_w.at[3]) if j == 0 and hf == 0 else None, fn)

    def ctx_m_block(j, hf):
        def fn():
            r = _nn(tm_scr[:, hf * HB:(hf + 1) * HB],
                    wuv_v[j * 4096 + hf * HB:j * 4096 + (hf + 1) * HB, :])
            acc(ctx_scr, ..., r, j == 0 and hf == 0)
        return a_block(None, fn)

    def flat_block():
        for k in range(H):
            cf_scr[:, k * D:(k + 1) * D] = jnp.broadcast_to(ctx_scr[k:k + 1, :], (8, D))
        if LASTR:
            crow = ctx_scr[H - 1:H, :].astype(BF16).astype(F32)
            sel = (lax.broadcasted_iota(jnp.int32, (LASTR, 128), 1)
                   == lax.broadcasted_iota(jnp.int32, (LASTR, 128), 0) + (128 - LASTR))
            ccol = jnp.sum(jnp.where(sel, crow, 0.0), axis=1, keepdims=True) * g_scr[0:1, 0:1]
            cb_scr[0:LASTR, :] = jnp.broadcast_to(ccol, (LASTR, 128))

    b_rounds = {SM_ROUND} | {2 * pos + 1 for pos in V_TRIG} | {2 * pos + 1 for pos in K_TRIG}
    free = [r for r in range(NR) if r not in b_rounds and r - 1 not in b_rounds]
    slots = A_SLOTS if A_SLOTS is not None else free[1::2]
    sched = {r: [] for r in range(NR)}

    def grp(fs):
        def f():
            for x in fs:
                x()
        return f

    def place(blocks, after_piece, start, allowed, group=AG):
        g = max(w_global_round(after_piece) + MARGIN, start)
        blocks = [grp(blocks[i:i + group]) for i in range(0, len(blocks), group)]
        for b in blocks:
            while g % NR not in allowed:
                g += 1
            assert g // NR < H - 1
            sched[g % NR].append((g // NR, b))
            g += 1
        return g

    g = place([qa_block(j, hf) for j in range(5) for hf in range(2)], wlo[2] - 1, 0, slots)
    g = place([blk for j in range(4) for blk in (qabs_t_block(j, 0), qabs_t_block(j, 1),
                                                 qabs_c_block(j, 0), qabs_c_block(j, 1))],
              wlo[3] - 1, g, slots)
    g = place([sc_block(j) for j in range(8)]
              + [a_block(None, sma_max), sma_exp(0), sma_exp(1)]
              + [cc_block(j) for j in range(8)], wlo[4] - 1, g, slots)
    g = place([blk for j in range(4) for blk in (ctx_e_block(j, 0), ctx_e_block(j, 1),
                                                 ctx_m_block(j, 0), ctx_m_block(j, 1))]
              + [a_block(None, flat_block)], wlo[5] - 1, g, slots)
    k_rest = 0
    while k_rest < H - WOA_TAIL:
        k1 = min(k_rest + PGRP, H - WOA_TAIL)
        last = wlo[5] + PPH * k1 - 1
        if last >= W_LOOP_END:
            break
        g2 = max(g, w_global_round(last) + MARGIN)
        while g2 % NR not in free:
            g2 += 1
        if g2 // NR >= H - 1:
            break
        sched[g2 % NR].append((g2 // NR, proj_a(k_rest, k1)))
        g = g2 + 1
        k_rest = k1

    PB = 128 // QROWS
    allseq = seq + main
    for i in range(NPRO):
        seq[i]().wait()
        if i + PD < len(allseq):
            allseq[i + PD]().start(priority=P1)
        if i >= NPRO - (DEPTH - PD) and DEPTH > PD:
            allseq[NPRO + PD + (i - (NPRO - (DEPTH - PD)))]().start(priority=P1)
        w_issue(i)
        if i in (0, 1):
            setup_r0(i)
        if i in (2, 3):
            setup_r0t(i - 2)
        if i == 4:
            setup_x()
        if PB - 1 <= i <= NQP and i % PB in (PB - 1, 0):
            qb_part((i - PB + 1) // PB, 0 if i % PB == PB - 1 else 1)
        for p in K_TRIG.get(i - NQP, []):
            qk_part(0, p)

    def body(h, carry):
        for r in range(NR):
            p1_copy(h, r).wait()
            if W_FIRST and r in W_ROUNDS:
                w_issue(W_BASE + h * NWR + W_ROUNDS.index(r))
            dh, r2 = divmod(r + DEPTH, NR)
            lim = H - 1 - dh if r2 % 2 == 0 else H - dh
            if lim >= H - 1:
                p1_copy(h + dh, r2).start(priority=P1)
            else:
                @pl.when(h < lim)
                def _():
                    p1_copy(h + dh, r2).start(priority=P1)
            if not W_FIRST and r in W_ROUNDS:
                w_issue(W_BASE + h * NWR + W_ROUNDS.index(r))
            if r == 0:
                wait_head_rows(wob_v, sem_wob, h)
            if r == SM_ROUND:
                softmax_b()
                proj_b(jnp.maximum(h - 1, 0))
            if r % 2 == 1:
                for p in K_TRIG.get(r // 2, []):
                    qk_part(h + 1, p)
                for p in V_TRIG.get(r // 2, []):
                    pv_part(h, p)
            if sched[r]:
                mask = sum(1 << hs for hs in {hs for hs, _ in sched[r]})

                @pl.when(jnp.bitwise_and(lax.shift_right_logical(jnp.int32(mask), h), 1) == 1)
                def _():
                    for hs, f in sched[r]:
                        pl.when(h == hs)(f)
        return carry

    lax.fori_loop(0, H - 1, body, 0)

    h = H - 1
    issued = set()
    for gidx in range(DEPTH, (H - 1) * NR + DEPTH):
        if gidx // NR == h and gidx % 2 == 1:
            issued.add((gidx % NR) // 2)
    for gidx in range(DEPTH):
        if gidx // NR == h and gidx % 2 == 1:
            issued.add((gidx % NR) // 2)
    pending = [j for j in range(NP) if j not in issued]

    SPLIT = H * D - LASTR

    def rows_copy(lo, hi, sem):
        return pltpu.make_async_copy(woa_hbm.at[pl.ds(lo, hi - lo)], woa_v.at[pl.ds(lo, hi - lo)], sem)

    def start_tail():
        for k in range(H - WOA_TAIL, H):
            if min((k + 1) * D, SPLIT) > k * D:
                rows_copy(k * D, min((k + 1) * D, SPLIT), sem_woa.at[k]).start(priority=P1)
        for u in range(NSUB if LASTR else 0):
            rows_copy(SPLIT + u * SUBR, SPLIT + (u + 1) * SUBR, sem_t.at[u]).start(priority=P1)

    if not pending:
        start_tail()
    wi = W_LOOP_END
    k_next = k_rest
    w_round = {}
    for j in range(NP):
        v_copy(h, VSEQ[j]).wait()
        if pending:
            v_copy(h, VSEQ[pending.pop(0)]).start(priority=P1)
            if not pending:
                start_tail()
        for _ in range(TAIL_W):
            if wi < NW:
                w_issue(wi)
                w_round[wi] = j
                wi += 1
        if j == 0:
            wait_head_rows(wob_v, sem_wob, h)
            softmax_b()
            proj_b(h - 1)
        if j in V_TRIG:
            for p in V_TRIG[j]:
                pv_part(h, p)
        elif j >= 1:
            k1 = k_next
            while (k1 < H - WOA_TAIL and k1 < k_next + PGRP and wlo[5] + PPH * (k1 + 1) - 1 < wi
                   and w_round.get(wlo[5] + PPH * (k1 + 1) - 1, -100) <= j - 4):
                k1 += 1
            if k1 > k_next:
                proj_a(k_next, k1)()
                k_next = k1
    assert wi >= NW
    proj_b(h)
    if k_next < H - WOA_TAIL:
        proj_a(k_next, H - WOA_TAIL)()
    for k in range(H - WOA_TAIL, H):
        lo, hi = k * D, min((k + 1) * D, SPLIT)
        if hi > lo:
            rows_copy(lo, hi, sem_woa.at[k]).wait()
            acca_scr[...] += _nn(cf_scr[:, lo:hi].astype(BF16), woa_v[lo:hi, :])

    g = g_scr[0:1, 0:1]
    part = g * acca_scr[0:1, :] + (1.0 - g) * accb_scr[0:1, :]
    if LASTR:
        accv = jnp.zeros((8, M), F32)
        for u in range(NSUB):
            lo = SPLIT + u * SUBR
            rows_copy(lo, lo + SUBR, sem_t.at[u]).wait()
            w = woa_v[lo:lo + SUBR, :].astype(F32)
            c = cb_scr[u * SUBR:(u + 1) * SUBR, :]
            prod = w * jnp.concatenate([c] * (M // 128), axis=1)
            for t in range(SUBR // 8):
                accv = accv + prod[t * 8:(t + 1) * 8, :]
        part = part + jnp.sum(accv, axis=0, keepdims=True)
    o_ref[0] = part.astype(o_ref.dtype)


@jax.jit
def pallas_gated_mix__compressed_kv_cla__gqa_block_cached__decode_kernel(
    A_x, A_c_kv, A_w_q, A_w_uk, A_w_uv, A_w_o, B_x, B_k_cache, B_v_cache, B_wq, B_wo, gate_w,
):
    del B_x
    ckv = A_c_kv.reshape(S, C)
    wqa = A_w_q.reshape(M * H, D)
    wuk = A_w_uk.reshape(C * H, D)
    wuv = A_w_uv.reshape(C * H, D)
    woa = A_w_o.reshape(H * D, M)
    k = B_k_cache.reshape(H, S, D)
    v = B_v_cache.reshape(H, S, D)

    any_spec = pl.BlockSpec(memory_space=pl.ANY)
    return pl.pallas_call(
        _kernel,
        in_specs=[any_spec] * 11,
        out_specs=pl.BlockSpec(memory_space=pltpu.VMEM),
        out_shape=jax.ShapeDtypeStruct((1, 1, M), BF16),
        scratch_shapes=[
            pltpu.VMEM((S, C), BF16),
            pltpu.VMEM((M * H, D), BF16),
            pltpu.VMEM((C * H, D), BF16),
            pltpu.VMEM((C * H, D), BF16),
            pltpu.VMEM((H * D, M), BF16),
            pltpu.VMEM((M, H * D), BF16),
            pltpu.VMEM((H * D, M), BF16),
            pltpu.VMEM((NB, S, D), BF16),
            pltpu.VMEM((NB, S, D), BF16),
            pltpu.VMEM((H, 8, D), F32),
            pltpu.VMEM((8, S), F32),
            pltpu.VMEM((8, S), F32),
            pltpu.VMEM((8, D), F32),
            pltpu.VMEM((8, D), F32),
            pltpu.VMEM((128, 4096), BF16),
            pltpu.VMEM((4096, 128), BF16),
            pltpu.VMEM((8, 4096), F32),
            pltpu.VMEM((H, D), F32),
            pltpu.VMEM((H, 4096), BF16),
            pltpu.VMEM((H, C), F32),
            pltpu.VMEM((H, S), F32),
            pltpu.VMEM((H, 128), F32),
            pltpu.VMEM((H, 128), F32),
            pltpu.VMEM((H, C), F32),
            pltpu.VMEM((H, D), F32),
            pltpu.VMEM((8, H * D), F32),
            pltpu.VMEM((8, M), F32),
            pltpu.VMEM((8, M), F32),
            pltpu.VMEM((8, 128), F32),
            pltpu.VMEM((128, 128), F32),
            pltpu.VMEM((1, 1, M), BF16),
            pltpu.VMEM((M,), BF16),
            pltpu.SemaphoreType.DMA((2,)),
            pltpu.SemaphoreType.DMA((NSUB,)),
            pltpu.SemaphoreType.DMA((PD,)),
            pltpu.SemaphoreType.DMA((NB * NP,)),
            pltpu.SemaphoreType.DMA((NB * NP,)),
            pltpu.SemaphoreType.DMA((4,)),
            pltpu.SemaphoreType.DMA((32,)),
            pltpu.SemaphoreType.DMA((32,)),
        ],
        compiler_params=pltpu.CompilerParams(vmem_limit_bytes=100 * 1024 * 1024,
                                             disable_bounds_checks=True,
                                             disable_semaphore_checks=True),
    )(A_x, gate_w, ckv, wqa, wuk, wuv, woa, k, v, B_wq, B_wo)
```

```python
import functools
import jax
import jax.numpy as jnp
from jax import lax
import jax.experimental.pallas as pl
import jax.experimental.pallas.tpu as pltpu

F32 = jnp.float32
BF16 = jnp.bfloat16

H = 32
D = 128
S = 4096
M = 640
C = 512
SCALE = float(D) ** -0.5


PCH = [320] * 10 + [256] + [320] * 2
POFF = [sum(PCH[:i]) for i in range(len(PCH))]
NP = len(PCH)
NR = 2 * NP
PARTS = [(0, 1280), (1280, 2560), (2560, 4096)]
VROT = 4
VSEQ = [(j + VROT) % NP for j in range(NP)]


def _triggers(order):
    trig = {}
    for p, (lo, hi) in enumerate(PARTS):
        need = [j for j in range(NP) if POFF[j] < hi and POFF[j] + PCH[j] > lo]
        trig.setdefault(max(order.index(j) for j in need), []).append(p)
    return trig


K_TRIG = _triggers(list(range(NP)))
V_TRIG = _triggers(VSEQ)
V_ORDER = [p for pos in sorted(V_TRIG) for p in V_TRIG[pos]]
DEPTH = NR
NB = 2
P0, P1 = 0, 1
WOA_TAIL = 4
QROWS = 8
NQP = M // QROWS
PD = 32
NPRO = NQP + NP
W_SKIP = (2, 9, 16, 23)
W_ROUNDS = [r for r in range(NR) if r not in W_SKIP]
NWR = len(W_ROUNDS)
WOP = 32
WQP = 128
WUP = 128
WCP = 32
TAIL_W = 1
SM_ROUND = 1
AG = 2
MARGIN = 8
PGRP = 3
LASTR = 128
NSUB = 4
SUBR = LASTR // NSUB


def _nt(a, b):
    return lax.dot_general(a, b, (((1,), (1,)), ((), ())), preferred_element_type=F32)


def _nn(a, b):
    return jnp.dot(a, b, preferred_element_type=F32)


def shr(k, n):
    return k >> n if isinstance(k, int) else lax.shift_right_logical(k, n)


def band(k, n):
    return k & n if isinstance(k, int) else jnp.bitwise_and(k, n)


def _kernel(xa_hbm, gw_hbm, ckv_hbm, wqa_hbm, wuk_hbm, wuv_hbm, woa_hbm,
            k_hbm, v_hbm, wqb_hbm, wob_hbm,
            o_ref,
            ckv_v, wqa_v, wuk_v, wuv_v, woa_v, wqb_v, wob_v,
            k_buf, v_buf, q_scr, s_scr, p_scr, l_scr, o_scr, r0_scr, r0t_scr, xe_scr,
            qa_scr, tm_scr, qabs_scr, sa_scr, ma_scr, la_scr, cc_scr, ctx_scr, cf_scr,
            acca_scr, accb_scr, g_scr, cb_scr, xa_v, gw_v,
            sem_s, sem_t, sem_q, sem_k, sem_v, sem_w, sem_wob, sem_woa):
    def k_copy(h, j):
        b = band(h, NB - 1)
        return pltpu.make_async_copy(k_hbm.at[h, pl.ds(POFF[j], PCH[j])],
                                     k_buf.at[b, pl.ds(POFF[j], PCH[j])], sem_k.at[b * NP + j])

    def v_copy(h, j):
        b = band(h, NB - 1)
        return pltpu.make_async_copy(v_hbm.at[h, pl.ds(POFF[j], PCH[j])],
                                     v_buf.at[b, pl.ds(POFF[j], PCH[j])], sem_v.at[b * NP + j])

    def row_piece(src, dst, k, rows, sem):
        return pltpu.make_async_copy(src.at[pl.ds(k * rows, rows)], dst.at[pl.ds(k * rows, rows)], sem)

    def wq_copy(i):
        return row_piece(wqb_hbm, wqb_v, i, QROWS, sem_q.at[i % PD])

    PPH = D // WOP
    SH = PPH.bit_length() - 1
    wtab = [
        (H * PPH, lambda k: row_piece(wob_hbm, wob_v, k, WOP, sem_wob.at[shr(k, SH)])),
        (M * H // WQP, lambda k: row_piece(wqa_hbm, wqa_v, k, WQP, sem_w.at[0])),
        (C * H // WUP, lambda k: row_piece(wuk_hbm, wuk_v, k, WUP, sem_w.at[1])),
        (S // WCP, lambda k: row_piece(ckv_hbm, ckv_v, k, WCP, sem_w.at[2])),
        (C * H // WUP, lambda k: row_piece(wuv_hbm, wuv_v, k, WUP, sem_w.at[3])),
        ((H - WOA_TAIL) * PPH, lambda k: row_piece(woa_hbm, woa_v, k, WOP, sem_woa.at[shr(k, SH)])),
    ]
    wlo = [sum(n for n, _ in wtab[:a]) for a in range(len(wtab) + 1)]
    NW = wlo[-1]
    W_BASE = NPRO
    W_LOOP_END = W_BASE + (H - 1) * NWR
    assert W_LOOP_END + NP * TAIL_W >= NW, (W_LOOP_END + NP * TAIL_W, NW)

    def w_global_round(i):
        k = i - W_BASE
        if k < 0:
            return -1
        return (k // NWR) * NR + W_ROUNDS[k % NWR]

    def w_issue(i):
        if isinstance(i, int):
            for a, (n, f) in enumerate(wtab):
                if wlo[a] <= i < wlo[a + 1]:
                    f(i - wlo[a]).start(priority=P0)
            return
        for a, (n, f) in enumerate(wtab):
            @pl.when(jnp.logical_and(i >= wlo[a], i < wlo[a + 1]))
            def _():
                f(i - wlo[a]).start(priority=P0)

    def wait_all(buf, sem):
        pltpu.make_async_copy(buf, buf, sem).wait()

    def wait_head_rows(w_v, sem, k):
        off = k * D if isinstance(k, int) else pl.multiple_of(k * D, D)
        blk = w_v.at[pl.ds(off, D)]
        pltpu.make_async_copy(blk, blk, sem.at[k]).wait()

    def p1_copy(h, r):
        return k_copy(h + 1, r // 2) if r % 2 == 0 else v_copy(h, VSEQ[r // 2])

    small = [pltpu.make_async_copy(xa_hbm, xa_v, sem_s.at[0]),
             pltpu.make_async_copy(gw_hbm, gw_v, sem_s.at[1])]
    seq = [functools.partial(wq_copy, i) for i in range(NQP)]
    seq += [functools.partial(k_copy, 0, j) for j in range(NP)]
    main = [functools.partial(p1_copy, g // NR, g % NR) for g in range(DEPTH)]
    for i in range(PD):
        seq[i]().start(priority=P1)
    for c in small:
        c.start(priority=P0)

    def hmask128():
        return (jnp.bitwise_and(lax.broadcasted_iota(jnp.int32, (H, 128), 1), H - 1)
                == lax.broadcasted_iota(jnp.int32, (H, 128), 0))

    def mask_heads(t):
        m = hmask128()
        return jnp.concatenate(
            [jnp.where(m, t[:, b * 128:(b + 1) * 128], 0.0) for b in range(t.shape[1] // 128)],
            axis=1).astype(BF16)

    def setup_r0(hf):
        cols = lax.broadcasted_iota(jnp.int32, (128, 2048), 1) + hf * 2048
        r0_scr[:, hf * 2048:(hf + 1) * 2048] = (
            lax.shift_right_logical(cols, 5)
            == lax.broadcasted_iota(jnp.int32, (128, 2048), 0)).astype(F32).astype(BF16)

    def setup_r0t(hf):
        rows = lax.broadcasted_iota(jnp.int32, (2048, 128), 0) + hf * 2048
        r0t_scr[hf * 2048:(hf + 1) * 2048, :] = (
            lax.shift_right_logical(rows, 5)
            == lax.broadcasted_iota(jnp.int32, (2048, 128), 1)).astype(F32).astype(BF16)

    def setup_x():
        acca_scr[...] = jnp.zeros((8, M), F32)
        accb_scr[...] = jnp.zeros((8, M), F32)
        o_scr[...] = jnp.zeros((8, D), F32)
        for c in small:
            c.wait()
        xa = xa_v[0].astype(F32)
        x8 = jnp.concatenate([xa[:, j * 128:(j + 1) * 128] for j in range(M // 128)]
                             + [jnp.zeros((3, 128), F32)], axis=0)
        xe_scr[...] = _nn(x8.astype(BF16), r0_scr[...])
        gw = gw_v[...].astype(F32).reshape(1, M)
        g = jax.nn.sigmoid(jnp.sum(xa * gw, axis=-1, keepdims=True))
        g_scr[...] = jnp.broadcast_to(g, (8, 128))

    def qb_part(blk, half):
        xb8 = jnp.broadcast_to(xa_v[0][:, blk * 128:(blk + 1) * 128].astype(F32), (8, 128)).astype(BF16)
        qb = _nn(xb8, wqb_v[blk * 128:(blk + 1) * 128, half * 2048:(half + 1) * 2048])
        for hh in range(16):
            if blk == 0:
                q_scr[half * 16 + hh] = qb[:, hh * D:(hh + 1) * D]
            else:
                q_scr[half * 16 + hh] += qb[:, hh * D:(hh + 1) * D]

    def qk_part(hn, part):
        lo, hi = PARTS[part]
        q = q_scr[hn].astype(BF16)
        s_scr[:, lo:hi] = _nt(q, k_buf[band(hn, NB - 1), lo:hi, :])

    def softmax_b():
        s = s_scr[...] * SCALE
        p = jnp.exp(s - jnp.max(s, axis=-1, keepdims=True))
        p_scr[...] = p
        l_scr[...] = jnp.broadcast_to(jnp.sum(p, axis=-1, keepdims=True), (8, D))

    def pv_part(h, part):
        lo, hi = PARTS[part]
        r = _nn(p_scr[:, lo:hi].astype(BF16), v_buf[band(h, NB - 1), lo:hi, :])
        if part == V_ORDER[0]:
            o_scr[...] = r
        elif part != V_ORDER[-1]:
            o_scr[...] += r
        else:
            o_scr[...] = (o_scr[...] + r) / l_scr[...]

    def proj_b(h):
        off = h * D if isinstance(h, int) else pl.multiple_of(h * D, D)
        accb_scr[...] += _nn(o_scr[...].astype(BF16), wob_v[pl.ds(off, D), :])

    def proj_a(k0, k1):
        def f():
            for k in range(k0, k1):
                wait_head_rows(woa_v, sem_woa, k)
            acca_scr[...] += _nn(cf_scr[:, k0 * D:k1 * D].astype(BF16), woa_v[k0 * D:k1 * D, :])
        return f

    HB = 2048

    def a_block(wait, fn):
        def f():
            if wait is not None:
                wait_all(*wait)
            fn()
        return f

    def acc(ref, idx, r, first):
        if first:
            ref[idx] = r
        else:
            ref[idx] += r

    def qa_block(j, hf):
        def fn():
            xsel = mask_heads(jnp.broadcast_to(xe_scr[j:j + 1, hf * HB:(hf + 1) * HB], (H, HB)))
            r = _nn(xsel, wqa_v[j * 4096 + hf * HB:j * 4096 + (hf + 1) * HB, :])
            acc(qa_scr, ..., r, j == 0 and hf == 0)
        return a_block((wqa_v, sem_w.at[0]) if j == 0 and hf == 0 else None, fn)

    def qabs_t_block(j, hf):
        def fn():
            t = _nt(qa_scr[...].astype(BF16), wuk_v[j * 4096 + hf * HB:j * 4096 + (hf + 1) * HB, :])
            tm_scr[:, hf * HB:(hf + 1) * HB] = mask_heads(t)
        return a_block((wuk_v, sem_w.at[1]) if j == 0 and hf == 0 else None, fn)

    def qabs_c_block(j, hf):
        def fn():
            r = _nn(tm_scr[:, hf * HB:(hf + 1) * HB], r0t_scr[hf * HB:(hf + 1) * HB, :])
            acc(qabs_scr, (slice(None), slice(j * 128, (j + 1) * 128)), r, hf == 0)
        return a_block(None, fn)

    def sc_block(j):
        def fn():
            sa_scr[:, j * 512:(j + 1) * 512] = _nt(qabs_scr[...].astype(BF16),
                                                   ckv_v[j * 512:(j + 1) * 512, :]) * SCALE
        return a_block((ckv_v, sem_w.at[2]) if j == 0 else None, fn)

    def sma_max():
        ma_scr[...] = jnp.broadcast_to(jnp.max(sa_scr[...], axis=-1, keepdims=True), (H, 128))

    def sma_exp(hf):
        def fn():
            pa = jnp.exp(sa_scr[:, hf * HB:(hf + 1) * HB] - ma_scr[:, 0:1])
            sa_scr[:, hf * HB:(hf + 1) * HB] = pa
            acc(la_scr, ..., jnp.broadcast_to(jnp.sum(pa, axis=-1, keepdims=True), (H, 128)), hf == 0)
        return a_block(None, fn)

    def cc_block(j):
        def fn():
            r = _nn(sa_scr[:, j * 512:(j + 1) * 512].astype(BF16), ckv_v[j * 512:(j + 1) * 512, :])
            acc(cc_scr, ..., r, j == 0)
        return a_block(None, fn)

    def ctx_e_block(j, hf):
        def fn():
            cc = (cc_scr[:, j * 128:(j + 1) * 128] / la_scr[...]).astype(BF16)
            tm_scr[:, hf * HB:(hf + 1) * HB] = mask_heads(_nn(cc, r0_scr[:, hf * HB:(hf + 1) * HB]))
        return a_block((wuv_v, sem_w.at[3]) if j == 0 and hf == 0 else None, fn)

    def ctx_m_block(j, hf):
        def fn():
            r = _nn(tm_scr[:, hf * HB:(hf + 1) * HB],
                    wuv_v[j * 4096 + hf * HB:j * 4096 + (hf + 1) * HB, :])
            acc(ctx_scr, ..., r, j == 0 and hf == 0)
        return a_block(None, fn)

    def flat_block():
        for k in range(H):
            cf_scr[:, k * D:(k + 1) * D] = jnp.broadcast_to(ctx_scr[k:k + 1, :], (8, D))
        if LASTR:
            crow = ctx_scr[H - 1:H, :].astype(BF16).astype(F32)
            sel = (lax.broadcasted_iota(jnp.int32, (LASTR, 128), 1)
                   == lax.broadcasted_iota(jnp.int32, (LASTR, 128), 0) + (128 - LASTR))
            ccol = jnp.sum(jnp.where(sel, crow, 0.0), axis=1, keepdims=True) * g_scr[0:1, 0:1]
            cb_scr[0:LASTR, :] = jnp.broadcast_to(ccol, (LASTR, 128))

    b_rounds = {SM_ROUND} | {2 * pos + 1 for pos in V_TRIG} | {2 * pos + 1 for pos in K_TRIG}
    free = [r for r in range(NR) if r not in b_rounds and r - 1 not in b_rounds]
    slots = free[1::2]
    sched = {r: [] for r in range(NR)}

    def grp(fs):
        def f():
            for x in fs:
                x()
        return f

    def place(blocks, after_piece, start, allowed, group=AG):
        g = max(w_global_round(after_piece) + MARGIN, start)
        blocks = [grp(blocks[i:i + group]) for i in range(0, len(blocks), group)]
        for b in blocks:
            while g % NR not in allowed:
                g += 1
            assert g // NR < H - 1
            sched[g % NR].append((g // NR, b))
            g += 1
        return g

    g = place([qa_block(j, hf) for j in range(5) for hf in range(2)], wlo[2] - 1, 0, slots)
    g = place([blk for j in range(4) for blk in (qabs_t_block(j, 0), qabs_t_block(j, 1),
                                                 qabs_c_block(j, 0), qabs_c_block(j, 1))],
              wlo[3] - 1, g, slots)
    g = place([sc_block(j) for j in range(8)]
              + [a_block(None, sma_max), sma_exp(0), sma_exp(1)]
              + [cc_block(j) for j in range(8)], wlo[4] - 1, g, slots)
    g = place([blk for j in range(4) for blk in (ctx_e_block(j, 0), ctx_e_block(j, 1),
                                                 ctx_m_block(j, 0), ctx_m_block(j, 1))]
              + [a_block(None, flat_block)], wlo[5] - 1, g, slots)
    k_rest = 0
    while k_rest < H - WOA_TAIL:
        k1 = min(k_rest + PGRP, H - WOA_TAIL)
        last = wlo[5] + PPH * k1 - 1
        if last >= W_LOOP_END:
            break
        g2 = max(g, w_global_round(last) + MARGIN)
        while g2 % NR not in free:
            g2 += 1
        if g2 // NR >= H - 1:
            break
        sched[g2 % NR].append((g2 // NR, proj_a(k_rest, k1)))
        g = g2 + 1
        k_rest = k1

    PB = 128 // QROWS
    allseq = seq + main
    for i in range(NPRO):
        seq[i]().wait()
        if i + PD < len(allseq):
            allseq[i + PD]().start(priority=P1)
        if i >= NPRO - (DEPTH - PD) and DEPTH > PD:
            allseq[NPRO + PD + (i - (NPRO - (DEPTH - PD)))]().start(priority=P1)
        w_issue(i)
        if i in (0, 1):
            setup_r0(i)
        if i in (2, 3):
            setup_r0t(i - 2)
        if i == 4:
            setup_x()
        if PB - 1 <= i <= NQP and i % PB in (PB - 1, 0):
            qb_part((i - PB + 1) // PB, 0 if i % PB == PB - 1 else 1)
        for p in K_TRIG.get(i - NQP, []):
            qk_part(0, p)

    def body(h, carry):
        for r in range(NR):
            p1_copy(h, r).wait()
            dh, r2 = divmod(r + DEPTH, NR)
            lim = H - 1 - dh if r2 % 2 == 0 else H - dh
            if lim >= H - 1:
                p1_copy(h + dh, r2).start(priority=P1)
            else:
                @pl.when(h < lim)
                def _():
                    p1_copy(h + dh, r2).start(priority=P1)
            if r in W_ROUNDS:
                w_issue(W_BASE + h * NWR + W_ROUNDS.index(r))
            if r == 0:
                wait_head_rows(wob_v, sem_wob, h)
            if r == SM_ROUND:
                softmax_b()
                proj_b(jnp.maximum(h - 1, 0))
            if r % 2 == 1:
                for p in K_TRIG.get(r // 2, []):
                    qk_part(h + 1, p)
                for p in V_TRIG.get(r // 2, []):
                    pv_part(h, p)
            if sched[r]:
                mask = sum(1 << hs for hs in {hs for hs, _ in sched[r]})

                @pl.when(jnp.bitwise_and(lax.shift_right_logical(jnp.int32(mask), h), 1) == 1)
                def _():
                    for hs, f in sched[r]:
                        pl.when(h == hs)(f)
        return carry

    lax.fori_loop(0, H - 1, body, 0)

    h = H - 1
    issued = set()
    for gidx in range(DEPTH, (H - 1) * NR + DEPTH):
        if gidx // NR == h and gidx % 2 == 1:
            issued.add((gidx % NR) // 2)
    for gidx in range(DEPTH):
        if gidx // NR == h and gidx % 2 == 1:
            issued.add((gidx % NR) // 2)
    pending = [j for j in range(NP) if j not in issued]

    SPLIT = H * D - LASTR

    def rows_copy(lo, hi, sem):
        return pltpu.make_async_copy(woa_hbm.at[pl.ds(lo, hi - lo)], woa_v.at[pl.ds(lo, hi - lo)], sem)

    def start_tail():
        for k in range(H - WOA_TAIL, H):
            if min((k + 1) * D, SPLIT) > k * D:
                rows_copy(k * D, min((k + 1) * D, SPLIT), sem_woa.at[k]).start(priority=P1)
        for u in range(NSUB if LASTR else 0):
            rows_copy(SPLIT + u * SUBR, SPLIT + (u + 1) * SUBR, sem_t.at[u]).start(priority=P1)

    if not pending:
        start_tail()
    wi = W_LOOP_END
    k_next = k_rest
    w_round = {}
    for j in range(NP):
        v_copy(h, VSEQ[j]).wait()
        if pending:
            v_copy(h, VSEQ[pending.pop(0)]).start(priority=P1)
            if not pending:
                start_tail()
        for _ in range(TAIL_W):
            if wi < NW:
                w_issue(wi)
                w_round[wi] = j
                wi += 1
        if j == 0:
            wait_head_rows(wob_v, sem_wob, h)
            softmax_b()
            proj_b(h - 1)
        if j in V_TRIG:
            for p in V_TRIG[j]:
                pv_part(h, p)
        elif j >= 1:
            k1 = k_next
            while (k1 < H - WOA_TAIL and k1 < k_next + PGRP and wlo[5] + PPH * (k1 + 1) - 1 < wi
                   and w_round.get(wlo[5] + PPH * (k1 + 1) - 1, -100) <= j - 4):
                k1 += 1
            if k1 > k_next:
                proj_a(k_next, k1)()
                k_next = k1
    assert wi >= NW
    proj_b(h)
    if k_next < H - WOA_TAIL:
        proj_a(k_next, H - WOA_TAIL)()
    for k in range(H - WOA_TAIL, H):
        lo, hi = k * D, min((k + 1) * D, SPLIT)
        if hi > lo:
            rows_copy(lo, hi, sem_woa.at[k]).wait()
            acca_scr[...] += _nn(cf_scr[:, lo:hi].astype(BF16), woa_v[lo:hi, :])

    g = g_scr[0:1, 0:1]
    part = g * acca_scr[0:1, :] + (1.0 - g) * accb_scr[0:1, :]
    if LASTR:
        accv = jnp.zeros((8, M), F32)
        for u in range(NSUB):
            lo = SPLIT + u * SUBR
            rows_copy(lo, lo + SUBR, sem_t.at[u]).wait()
            w = woa_v[lo:lo + SUBR, :].astype(F32)
            c = cb_scr[u * SUBR:(u + 1) * SUBR, :]
            prod = w * jnp.concatenate([c] * (M // 128), axis=1)
            for t in range(SUBR // 8):
                accv = accv + prod[t * 8:(t + 1) * 8, :]
        part = part + jnp.sum(accv, axis=0, keepdims=True)
    o_ref[0] = part.astype(o_ref.dtype)


@jax.jit
def pallas_gated_mix__compressed_kv_cla__gqa_block_cached__decode_kernel(
    A_x, A_c_kv, A_w_q, A_w_uk, A_w_uv, A_w_o, B_x, B_k_cache, B_v_cache, B_wq, B_wo, gate_w,
):
    del B_x
    ckv = A_c_kv.reshape(S, C)
    wqa = A_w_q.reshape(M * H, D)
    wuk = A_w_uk.reshape(C * H, D)
    wuv = A_w_uv.reshape(C * H, D)
    woa = A_w_o.reshape(H * D, M)
    k = B_k_cache.reshape(H, S, D)
    v = B_v_cache.reshape(H, S, D)

    any_spec = pl.BlockSpec(memory_space=pl.ANY)
    return pl.pallas_call(
        _kernel,
        in_specs=[any_spec] * 11,
        out_specs=pl.BlockSpec(memory_space=pltpu.VMEM),
        out_shape=jax.ShapeDtypeStruct((1, 1, M), BF16),
        scratch_shapes=[
            pltpu.VMEM((S, C), BF16),
            pltpu.VMEM((M * H, D), BF16),
            pltpu.VMEM((C * H, D), BF16),
            pltpu.VMEM((C * H, D), BF16),
            pltpu.VMEM((H * D, M), BF16),
            pltpu.VMEM((M, H * D), BF16),
            pltpu.VMEM((H * D, M), BF16),
            pltpu.VMEM((NB, S, D), BF16),
            pltpu.VMEM((NB, S, D), BF16),
            pltpu.VMEM((H, 8, D), F32),
            pltpu.VMEM((8, S), F32),
            pltpu.VMEM((8, S), F32),
            pltpu.VMEM((8, D), F32),
            pltpu.VMEM((8, D), F32),
            pltpu.VMEM((128, 4096), BF16),
            pltpu.VMEM((4096, 128), BF16),
            pltpu.VMEM((8, 4096), F32),
            pltpu.VMEM((H, D), F32),
            pltpu.VMEM((H, 4096), BF16),
            pltpu.VMEM((H, C), F32),
            pltpu.VMEM((H, S), F32),
            pltpu.VMEM((H, 128), F32),
            pltpu.VMEM((H, 128), F32),
            pltpu.VMEM((H, C), F32),
            pltpu.VMEM((H, D), F32),
            pltpu.VMEM((8, H * D), F32),
            pltpu.VMEM((8, M), F32),
            pltpu.VMEM((8, M), F32),
            pltpu.VMEM((8, 128), F32),
            pltpu.VMEM((128, 128), F32),
            pltpu.VMEM((1, 1, M), BF16),
            pltpu.VMEM((M,), BF16),
            pltpu.SemaphoreType.DMA((2,)),
            pltpu.SemaphoreType.DMA((NSUB,)),
            pltpu.SemaphoreType.DMA((PD,)),
            pltpu.SemaphoreType.DMA((NB * NP,)),
            pltpu.SemaphoreType.DMA((NB * NP,)),
            pltpu.SemaphoreType.DMA((4,)),
            pltpu.SemaphoreType.DMA((32,)),
            pltpu.SemaphoreType.DMA((32,)),
        ],
        compiler_params=pltpu.CompilerParams(vmem_limit_bytes=100 * 1024 * 1024,
                                             disable_bounds_checks=True,
                                             disable_semaphore_checks=True),
    )(A_x, gate_w, ckv, wqa, wuk, wuv, woa, k, v, B_wq, B_wo)
```
